```python
import os as _os
_os.environ.setdefault("JAX_PLATFORMS", "cpu")
import jax
import jax.numpy as jnp

def _softmax(x, axis=-1):
    return jax.nn.softmax(x, axis=axis)
def _gelu(x):
    return jax.nn.gelu(x, approximate=True)
def _silu(x):
    return jax.nn.silu(x)
def _sigmoid(x):
    return jax.nn.sigmoid(x)
def _layernorm(x, axis=-1, eps=1e-5):
    m = jnp.mean(x, axis=axis, keepdims=True)
    v = jnp.var(x, axis=axis, keepdims=True)
    return (x - m) / jnp.sqrt(v + eps)
def _scatter_add(tgt, idx, src, axis=0):
    return tgt.at[idx].add(src)
def _segment_sum(src, seg, n):
    return jax.ops.segment_sum(src, seg, n)
class _Rng:
    def __init__(self, key):
        self._k = key
    def _next(self):
        self._k, sub = jax.random.split(self._k)
        return sub
    def normal(self, shape):
        return jax.random.normal(self._next(), shape, dtype=jnp.bfloat16)
    def randint(self, lo, hi, shape):
        return jax.random.randint(self._next(), shape, lo, hi, dtype=jnp.int32)
    def uniform(self, shape, lo=0.0, hi=1.0):
        return jax.random.uniform(self._next(), shape, jnp.bfloat16, lo, hi)
    def permutation(self, n):
        return jax.random.permutation(self._next(), n)


kernel_name = 'concat_heads__compressed_kv_cla__gqa_block_cached__decode'

def setup_inputs():
    _rng = _Rng(jax.random.key(int.from_bytes(__import__("os").urandom(4), "little")))
    _w = (lambda a: (lambda t: t.astype(jnp.bfloat16) if jnp.issubdtype(t.dtype, jnp.floating) else t)(jnp.asarray(a)))
    def _A_setup():
        B, H, Sq, Sk, D, M = 4, 32, 1, 4096, 128, 512
        Dc = 4 * D
        return {
            "x": _w((lambda *s: _rng.normal(s) * 3.2)(B, Sq, M)),
            "c_kv": _w((lambda *s: _rng.normal(s) * 0.05)(B, Sk, Dc)),
            "w_q": _w((lambda *s: _rng.normal(s) * 3.2)(M, H, D) * (M ** -0.5)),
            "w_uk": _w((lambda *s: _rng.normal(s) * 3.2)(Dc, H, D) * (Dc ** -0.5)),
            "w_uv": _w((lambda *s: _rng.normal(s) * 0.05)(Dc, H, D) * (Dc ** -0.5)),
            "w_o": _w((lambda *s: _rng.normal(s) * 0.05)(H, D, M) * ((H * D) ** -0.5)),
        }
    _A_in = _A_setup()

    def _B_setup():
        B, Sq, D = 4, 1, 512
        Hq, Hkv, Sk, Dh = 32, 8, 4096, 128
        assert Hq % Hkv == 0, (Hq, Hkv)
        return {
            "x": _w((lambda *s: _rng.normal(s) * 0.8)(B, Sq, D)),
            "k_cache": _w((lambda *s: _rng.normal(s) * 0.8)(B, Hkv, Sk, Dh)),
            "v_cache": _w((lambda *s: _rng.normal(s) * 0.05)(B, Hkv, Sk, Dh)),
            "wq": _w((lambda *s: _rng.normal(s) * 0.8)(D, Hq * Dh) * (D ** -0.5)),
            "wo": _w((lambda *s: _rng.normal(s) * 0.05)(Hq * Dh, D) * ((Hq * Dh) ** -0.5)),
        }
    _B_in = _B_setup()

    return {
        "A_x": _A_in["x"],
        "A_c_kv": _A_in["c_kv"],
        "A_w_q": _A_in["w_q"],
        "A_w_uk": _A_in["w_uk"],
        "A_w_uv": _A_in["w_uv"],
        "A_w_o": _A_in["w_o"],
        "B_x": _B_in["x"],
        "B_k_cache": _B_in["k_cache"],
        "B_v_cache": _B_in["v_cache"],
        "B_wq": _B_in["wq"],
        "B_wo": _B_in["wo"],
    }

def reference(A_x, A_c_kv, A_w_q, A_w_uk, A_w_uv, A_w_o, B_x, B_k_cache, B_v_cache, B_wq, B_wo):
    def _A_ref(x, c_kv, w_q, w_uk, w_uv, w_o):
        B, Sq, M = x.shape[0], x.shape[1], x.shape[2]
        Sk = c_kv.shape[1]
        H, D = w_q.shape[1], w_q.shape[2]
        q = jnp.einsum("bqm,mhd->bhqd", x, w_q)
        k = jnp.einsum("bkc,chd->bhkd", c_kv, w_uk)
        v = jnp.einsum("bkc,chd->bhkd", c_kv, w_uv)
        scores = jnp.einsum("bhqd,bhkd->bhqk", q, k) * (D ** -0.5)
        off = Sk - Sq
        qi = jnp.arange(Sq)[:, None]
        kj = jnp.arange(Sk)[None, :]
        cmask = kj <= (qi + off)
        scores = jnp.where(cmask[None, None], scores, -1e9)
        p = _softmax(scores, axis=-1)
        ctx = jnp.einsum("bhqk,bhkd->bhqd", p, v)
        return jnp.einsum("bhqd,hdm->bqm", ctx, w_o)

    def _B_ref(x, k_cache, v_cache, wq, wo):
        B, Sq, D = x.shape
        Hq, Dh = 32, 128
        Hkv = k_cache.shape[1]
        rep = Hq // Hkv
        q = (lambda x, *d: x.transpose(*d))((x @ wq).reshape(B, Sq, Hq, Dh), 0, 2, 1, 3)
        k = jnp.repeat(k_cache, rep, axis=1)
        v = jnp.repeat(v_cache, rep, axis=1)
        scores = jnp.einsum("bhqd,bhkd->bhqk", q, k) * (Dh ** -0.5)
        p = _softmax(scores, axis=-1)
        o = jnp.einsum("bhqk,bhkd->bhqd", p, v)
        return (lambda x, *d: x.transpose(*d))(o, 0, 2, 1, 3).reshape(B, Sq, Hq * Dh) @ wo

    a = _A_ref(A_x, A_c_kv, A_w_q, A_w_uk, A_w_uv, A_w_o)
    b = _B_ref(B_x, B_k_cache, B_v_cache, B_wq, B_wo)
    return jnp.concatenate([a, b], axis=-1)
```

```python
import jax
import jax.numpy as jnp
from jax import lax
import jax.experimental.pallas as pl
import jax.experimental.pallas.tpu as pltpu

B, H, SK, D, M = 4, 32, 4096, 128, 512
DC = 512
HKV = 8
NPAIR = B * HKV
F32 = jnp.float32
BF16 = jnp.bfloat16
WO_CHUNKS = [(0, 2048), (2048, 1024), (3072, 512), (3584, 256), (3840, 128), (3968, 128)]
NT = (((1,), (1,)), ((), ()))
NN = (((1,), (0,)), ((), ()))


def _split_pair(w_u32):
    lo = pltpu.bitcast(w_u32 << 16, F32).astype(BF16)
    hi = pltpu.bitcast(w_u32 & jnp.uint32(0xFFFF0000), F32).astype(BF16)
    return lo, hi


def kernel(ax_hbm, ckv_hbm, awq_hbm, awuk_hbm, awuv_hbm, awo_hbm, bx_hbm, k_hbm, v_hbm, bwq_hbm, bwo_hbm,
           out_ref,
           ax_buf, bx_buf, ckv_buf, awq_buf, awuk_buf, awuv_buf, awo_buf, k_buf, v_buf, bwq_buf, bwo_buf,
           qa_scr, ctx_scr, ctxh_scr, qb_scr, ob_scr,
           sems):
    scale = D ** -0.5
    cp_ax = pltpu.make_async_copy(ax_hbm, ax_buf, sems.at[0])
    cp_bx = pltpu.make_async_copy(bx_hbm, bx_buf, sems.at[1])
    cp_awq = pltpu.make_async_copy(awq_hbm, awq_buf, sems.at[2])
    cp_awuk = pltpu.make_async_copy(awuk_hbm, awuk_buf, sems.at[3])
    cp_awuv = pltpu.make_async_copy(awuv_hbm, awuv_buf, sems.at[4])
    cp_awo = pltpu.make_async_copy(awo_hbm, awo_buf, sems.at[5])
    cp_bwq = pltpu.make_async_copy(bwq_hbm, bwq_buf, sems.at[6])

    def cp_bwo(i):
        r0, n = WO_CHUNKS[i]
        return pltpu.make_async_copy(bwo_hbm.at[pl.ds(r0, n)], bwo_buf.at[pl.ds(r0, n)], sems.at[43 + i])

    def cp_c(b):
        return pltpu.make_async_copy(ckv_hbm.at[b], ckv_buf.at[b], sems.at[7 + b])

    def cp_k(j):
        return pltpu.make_async_copy(k_hbm.at[pl.ds(2 * j, 2)], k_buf.at[pl.ds(2 * j, 2)], sems.at[11 + j])

    def cp_v(j):
        return pltpu.make_async_copy(v_hbm.at[pl.ds(2 * j, 2)], v_buf.at[pl.ds(2 * j, 2)], sems.at[27 + j])

    cp_ax.start()
    cp_bx.start()
    cp_awq.start()
    cp_awuk.start()
    for b in range(B):
        cp_c(b).start()
    cp_bwq.start()
    for j in range(NPAIR // 2):
        cp_k(j).start()
        cp_v(j).start()
    cp_awuv.start()
    cp_awo.start()
    for i in range(len(WO_CHUNKS)):
        cp_bwo(i).start()

    def load_x(buf):
        return buf[...]

    cp_ax.wait()
    cp_awq.wait()
    cp_awuk.wait()
    xa = load_x(ax_buf)
    awq32 = awq_buf.bitcast(jnp.uint32)
    awuk32 = awuk_buf.bitcast(jnp.uint32)

    def qa_body(jj, c):
        j0 = pl.multiple_of(4 * jj, 4)
        h0 = pl.multiple_of(8 * jj, 8)
        wv = awq32.at[pl.ds(j0, M * 16 - 12), :]
        uv = awuk32.at[pl.ds(j0, DC * 16 - 12), :]
        qv = qa_scr.at[:, pl.ds(h0, B * H - 24), :]
        for r in range(4):
            wlo, whi = _split_pair(wv[pl.ds(r, M, stride=16), :])
            ulo, uhi = _split_pair(uv[pl.ds(r, DC, stride=16), :])
            for p, (w, u) in enumerate(((wlo, ulo), (whi, uhi))):
                q = lax.dot_general(xa, w, NN, preferred_element_type=F32).astype(BF16)
                qa = lax.dot_general(q, u, NT, preferred_element_type=F32) * scale
                for cc in range(4):
                    qv[cc, pl.ds(2 * r + p, B, stride=H), :] = qa[:, cc * 128:(cc + 1) * 128]
        return c

    lax.fori_loop(0, 4, qa_body, 0)

    def a_body(b, c):
        cp_c(b).wait()
        r0 = pl.multiple_of(b * H, H)
        qa = jnp.concatenate([qa_scr[cc, pl.ds(r0, H), :] for cc in range(4)], axis=1).astype(BF16)
        ckv = ckv_buf[b]
        s = lax.dot_general(qa, ckv, NT, preferred_element_type=F32)
        m = jnp.max(s, axis=1, keepdims=True)
        p = jnp.exp(s - m)
        l = jnp.sum(p, axis=1, keepdims=True)
        ctx = lax.dot_general(p.astype(BF16), ckv, NN, preferred_element_type=F32) / l
        for cc in range(4):
            ctx_scr[cc, pl.ds(r0, H), :] = ctx[:, cc * 128:(cc + 1) * 128]
        return c

    lax.fori_loop(0, B, a_body, 0)

    cp_bx.wait()
    cp_bwq.wait()
    xb = load_x(bx_buf)
    qb = lax.dot_general(xb, bwq_buf[...], NN, preferred_element_type=F32)
    for h in range(H):
        qb_scr[pl.ds(h, B, stride=H), :] = qb[:, h * D:(h + 1) * D]

    row = lax.broadcasted_iota(jnp.int32, (8, 1), 0)

    def b_body(j, c):
        cp_k(j).wait()
        r0 = pl.multiple_of(j * 8, 8)
        q8 = qb_scr[pl.ds(r0, 8), :].astype(BF16)
        s0 = lax.dot_general(q8, k_buf[2 * j], NT, preferred_element_type=F32)
        s1 = lax.dot_general(q8, k_buf[2 * j + 1], NT, preferred_element_type=F32)
        s = jnp.where(row < 4, s0, s1) * scale
        m = jnp.max(s, axis=1, keepdims=True)
        p = jnp.exp(s - m)
        l = jnp.sum(p, axis=1, keepdims=True)
        pb = p.astype(BF16)
        cp_v(j).wait()
        o0 = lax.dot_general(pb, v_buf[2 * j], NN, preferred_element_type=F32)
        o1 = lax.dot_general(pb, v_buf[2 * j + 1], NN, preferred_element_type=F32)
        ob_scr[pl.ds(r0, 8), :] = jnp.where(row < 4, o0, o1) / l
        return c

    lax.fori_loop(0, NPAIR // 2, b_body, 0)

    cp_awuv.wait()
    awuv32 = awuv_buf.bitcast(jnp.uint32)

    def uv_body(jj, c):
        j0 = pl.multiple_of(4 * jj, 4)
        h0 = pl.multiple_of(8 * jj, 8)
        uv = awuv32.at[pl.ds(j0, DC * 16 - 12), :]
        cv = ctx_scr.at[:, pl.ds(h0, B * H - 24), :]
        for r in range(4):
            ulo, uhi = _split_pair(uv[pl.ds(r, DC, stride=16), :])
            for p, u in enumerate((ulo, uhi)):
                hh = 2 * r + p
                cc_rows = jnp.concatenate([cv[cc, pl.ds(hh, B, stride=H), :] for cc in range(4)], axis=1).astype(BF16)
                ctxh_scr[h0 + hh] = lax.dot_general(cc_rows, u, NN, preferred_element_type=F32)
        return c

    lax.fori_loop(0, 4, uv_body, 0)
    ctx_all = jnp.concatenate([ctxh_scr[h] for h in range(H)], axis=1).astype(BF16)
    cp_awo.wait()
    oa = lax.dot_general(ctx_all, awo_buf[...], NN, preferred_element_type=F32)

    ob_all = jnp.concatenate([ob_scr[pl.ds(h, B, stride=H), :] for h in range(H)], axis=1).astype(BF16)
    ob = None
    for i, (r0, n) in enumerate(WO_CHUNKS):
        cp_bwo(i).wait()
        part = lax.dot_general(ob_all[:, r0:r0 + n], bwo_buf[pl.ds(r0, n), :], NN, preferred_element_type=F32)
        ob = part if ob is None else ob + part
    res = jnp.concatenate([oa, ob], axis=1)
    out_ref[...] = res.astype(BF16)


@jax.jit
def pallas_concat_heads__compressed_kv_cla__gqa_block_cached__decode_kernel(A_x, A_c_kv, A_w_q, A_w_uk, A_w_uv, A_w_o, B_x, B_k_cache, B_v_cache, B_wq, B_wo):
    args = (
        A_x.reshape(B, M), A_c_kv,
        A_w_q.reshape(M * H, D), A_w_uk.reshape(DC * H, D), A_w_uv.reshape(DC * H, D),
        A_w_o.reshape(H * D, M),
        B_x.reshape(B, M), B_k_cache.reshape(NPAIR, SK, D), B_v_cache.reshape(NPAIR, SK, D), B_wq, B_wo,
    )
    scratch = [
        pltpu.VMEM((B, M), BF16), pltpu.VMEM((B, M), BF16),
        pltpu.VMEM((B, SK, DC), BF16),
        pltpu.VMEM((M * H, D), BF16), pltpu.VMEM((DC * H, D), BF16), pltpu.VMEM((DC * H, D), BF16),
        pltpu.VMEM((H * D, M), BF16),
        pltpu.VMEM((NPAIR, SK, D), BF16), pltpu.VMEM((NPAIR, SK, D), BF16),
        pltpu.VMEM((M, H * D), BF16), pltpu.VMEM((H * D, M), BF16),
        pltpu.VMEM((4, B * H, 128), F32), pltpu.VMEM((4, B * H, 128), F32),
        pltpu.VMEM((H, B, D), F32),
        pltpu.VMEM((B * H, D), F32), pltpu.VMEM((B * H, D), F32),
        pltpu.SemaphoreType.DMA((43 + len(WO_CHUNKS),)),
    ]
    return pl.pallas_call(
        kernel,
        in_specs=[pl.BlockSpec(memory_space=pl.ANY)] * 11,
        out_specs=pl.BlockSpec(memory_space=pltpu.VMEM),
        out_shape=jax.ShapeDtypeStruct((B, 2 * M), BF16),
        scratch_shapes=scratch,
        compiler_params=pltpu.CompilerParams(vmem_limit_bytes=122 * 1024 * 1024,
                                             disable_semaphore_checks=True, disable_bounds_checks=True),
    )(*args).reshape(B, 1, 2 * M)
```

```python
import jax
import jax.numpy as jnp
from jax import lax
import jax.experimental.pallas as pl
import jax.experimental.pallas.tpu as pltpu

B, H, SK, D, M = 4, 32, 4096, 128, 512
DC = 512
HKV = 8
NG = B * HKV
KB = 256
NSTEP = SK // KB
F32 = jnp.float32
BF16 = jnp.bfloat16
NT = (((1,), (1,)), ((), ()))
NN = (((1,), (0,)), ((), ()))
SEG = 32 * 1024
NS = 8

SCOPES = 0
NOCOMP = 0
NREM = 0
NREMU = 10
NV = 64
NW = 128
T_W = 11
T_A = 31
T_BQ = 9
T_B = 20
T_G = 6
LEAD = 10
LA = 36
NL = 20
CH = 16
XKV = 0
XD = 0

(S_AX, S_BX, S_BWQ, S_AWQ, S_AWUK, S_AWUV, S_C, S_K, S_V, S_AO, S_BO) = (0, 1, 2, 3, 4, 5, 6, 10, 12, 14, 21)
AO_LAST = [(0, 4), (4, 2), (6, 1), (7, 1)]
NSEM = S_BO + 4


def _dot(a, b, dn):
    if NOCOMP:
        n = b.shape[0] if dn == NT else b.shape[1]
        return (lax.broadcasted_iota(jnp.int32, (a.shape[0], n), 0) + lax.broadcasted_iota(jnp.int32, (a.shape[0], n), 1)).astype(F32)
    return lax.dot_general(a, b, dn, preferred_element_type=F32)


def _lag(t, extra):
    u = t.astype(jnp.uint32)
    for k in range(NREMU):
        u = lax.rem(u, jnp.uint32(900001 - 14 * k))
        if k < extra:
            u = u + jnp.uint32(1)
    if extra:
        u = u - jnp.uint32(min(extra, NREMU))
    return u.astype(jnp.int32)


def _split_pair(w_u32):
    lo = pltpu.bitcast(w_u32 << 16, F32).astype(BF16)
    hi = pltpu.bitcast(w_u32 & jnp.uint32(0xFFFF0000), F32).astype(BF16)
    return lo, hi


def kernel(ax_hbm, ckv_hbm, awq_hbm, awuk_hbm, awuv_hbm, awo_hbm, bx_hbm, k_hbm, v_hbm, bwq_hbm, bwo_hbm,
           out_ref,
           ax_buf, bx_buf, bwq_buf, awq_buf, awuk_buf, awuv_buf, c0_buf, c1_buf, c2_buf, c3_buf,
           k0_buf, k1_buf, v0_buf, v1_buf,
           ao0, ao1, ao2, ao3a, ao3b, ao3c, ao3d, bo0, bo1, bo2, bo3,
           q_scr, qa_scr, ctx_scr, ctxh_scr, qb_scr, m_scr, l_scr, acc_scr, sems):
    scale = D ** -0.5
    c_bufs = (c0_buf, c1_buf, c2_buf, c3_buf)
    k_bufs = (k0_buf, k1_buf)
    v_bufs = (v0_buf, v1_buf)
    zero = jnp.int32(0)

    def scoped(name, fn):
        if SCOPES:
            with jax.named_scope(name):
                return fn()
        return fn()

    class Load:
        def __init__(self, src, dst, sem, nfg=0, s0=0, r0=0):
            self.src, self.dst, self.sem, self.nfg, self.s0, self.r0 = src, dst, sem, nfg, s0, r0
            self.S, self.L, W = dst.shape
            self.seg = SEG // (W * 2)

        def copy(self, s, ns, r, nr):
            return pltpu.make_async_copy(self.src.at[pl.ds(self.s0 + s, ns), pl.ds(self.r0 + r, nr)],
                                         self.dst.at[pl.ds(s, ns), pl.ds(r, nr)], sems.at[self.sem])

        def bg(self):
            out = []
            for rnd in range(self.nfg // self.S, self.L // self.seg):
                s = max(self.nfg - rnd * self.S, 0)
                out.append((self.copy(s, self.S - s, rnd * self.seg, self.seg), self.S - s))
            return out

        def wait(self):
            scoped("wait", lambda: self.copy(0, self.S, 0, self.L).wait())

        def tick(self, t):
            s = lax.bitwise_and(t, self.S - 1)
            r = pl.multiple_of(lax.shift_right_logical(t, self.S.bit_length() - 1) * self.seg, self.seg)
            self.copy(s, 1, r, self.seg).start(priority=0)
            return _lag(t + 1, XKV if self.S == NG else XD)

    class Sched:
        def __init__(self):
            self.q, self.issued, self.ticks, self.rate = [], 0, 0, (256 - NW) / NW

        def feed(self, upto):
            while self.q and self.issued < (upto + LA) * self.rate:
                c, n = self.q.pop(0)
                c.start(priority=1)
                self.issued += n

        def ticks_(self, ld, t, n):
            for _ in range(n):
                self.feed(self.ticks)
                t = ld.tick(t)
                self.ticks += 1
            return t

        def pump(self, ld, t, n):
            while n > 0:
                k = n if (n <= CH + 4 or not self.q) else CH
                self.feed(self.ticks + k // 2)
                t = scoped(f"pump{k}", lambda: lax.fori_loop(0, k, lambda i, t: ld.tick(t), t))
                self.ticks += k
                n -= k
            return t

    cp_ax = pltpu.make_async_copy(ax_hbm, ax_buf, sems.at[S_AX])
    cp_bx = pltpu.make_async_copy(bx_hbm, bx_buf, sems.at[S_BX])
    awq = Load(awq_hbm, awq_buf, S_AWQ, NW)
    awuk = Load(awuk_hbm, awuk_buf, S_AWUK)
    awuv = Load(awuv_hbm, awuv_buf, S_AWUV, NW)
    ckv = [Load(ckv_hbm, c_bufs[b], S_C + b, NW if b % 2 else 0, s0=b * NS) for b in range(B)]
    HC = H * D // 2
    BQ = 0
    if BQ == 0:
        bwq_bg = [(pltpu.make_async_copy(bwq_hbm.at[:, pl.ds(r, 16)], bwq_buf.at[:, pl.ds(r, 16)], sems.at[S_BWQ]), 32)
                  for r in range(0, M // NS, 16)]
    else:
        bwq_bg = [(pltpu.make_async_copy(bwq_hbm.at[:, pl.ds(r, 8), pl.ds(c * HC, HC)],
                                         bwq_buf.at[:, pl.ds(r, 8), pl.ds(c * HC, HC)], sems.at[S_BWQ]), 8)
                  for r in range(0, M // NS, 8) for c in range(2)]
    ao = [Load(awo_hbm, buf, S_AO + g, r0=g * D) for g, buf in enumerate((ao0, ao1, ao2))]
    ao_last = [Load(awo_hbm, buf, S_AO + 3 + i, s0=AO_LAST[i][0], r0=3 * D) for i, buf in enumerate((ao3a, ao3b, ao3c, ao3d))]
    bo = [Load(bwo_hbm, buf, S_BO + g, 32 if g < 3 else NL, r0=g * D) for g, buf in enumerate((bo0, bo1, bo2, bo3))]

    def key0(j):
        return j * KB if isinstance(j, int) else pl.multiple_of(j * KB, KB)

    def kc(j, par):
        return Load(k_hbm, k_bufs[par], S_K + par, r0=key0(j))

    def vc(j, par):
        return Load(v_hbm, v_bufs[par], S_V + par, NV, r0=key0(j))

    sch = Sched()
    uk_bg = awuk.bg()
    sch.q = (uk_bg[:1] + [(cp_ax, 0), (cp_bx, 0)] + uk_bg[1:] + awq.bg() + ckv[0].bg() + ckv[1].bg() + ckv[2].bg() + ckv[3].bg()
             + bwq_bg + awuv.bg() + kc(0, 0).bg() + vc(0, 0).bg() + kc(1, 1).bg() + vc(1, 1).bg())

    sch.pump(awq, zero, NW)

    def weight_phase(st, t, w_buf, fn):
        w32 = w_buf.bitcast(jnp.uint32)
        for jj in range(4):
            t = sch.ticks_(st, t, T_W)
            for j in range(4 * jj, 4 * jj + 4):
                w = w32[:, pl.ds(j, M // NS, stride=16), :].reshape(M, D)
                for p, wp in enumerate(_split_pair(w)):
                    fn(2 * j + p, wp)
        return t

    st = ckv[1]
    t = sch.pump(st, zero, LEAD)
    cp_ax.wait()
    awq.wait()
    awuk.wait()

    def q_fn(h, w):
        q_scr[h] = _dot(ax_buf[...], w, NN)

    t = weight_phase(st, t, awq_buf, q_fn)
    t = sch.pump(st, t, 2)

    def qa_fn(h, u):
        qa = _dot(q_scr[h].astype(BF16), u, NT) * scale
        for cc in range(4):
            qa_scr[cc, pl.ds(h, B, stride=H), :] = qa[:, cc * 128:(cc + 1) * 128]

    t = weight_phase(st, t, awuk_buf, qa_fn)
    sch.pump(st, t, NW - LEAD - 8 * T_W - 2)

    def a_block(st, t, b):
        t = sch.ticks_(st, t, T_A)
        h0 = b * H
        qa = jnp.concatenate([qa_scr[cc, pl.ds(h0, H), :] for cc in range(4)], axis=1).astype(BF16)
        c = c_bufs[b][...].reshape(SK, DC)
        s = _dot(qa, c, NT)
        m = jnp.max(s, axis=1, keepdims=True)
        p = jnp.exp(s - m)
        l = jnp.sum(p, axis=1, keepdims=True)
        ctx = _dot(p.astype(BF16), c, NN) / l
        for cc in range(4):
            ctx_scr[cc, pl.ds(h0, H), :] = ctx[:, cc * 128:(cc + 1) * 128]
        return t

    for st, b0 in ((ckv[3], 0), (awuv, 2)):
        t = sch.pump(st, zero, LEAD)
        ckv[b0].wait()
        ckv[b0 + 1].wait()
        t = a_block(st, t, b0)
        t = sch.pump(st, t, 2)
        t = a_block(st, t, b0 + 1)
        sch.pump(st, t, NW - LEAD - 2 * T_A - 2)

    st = vc(0, 0)
    lead0 = NV - T_BQ - 4 * T_W
    t = sch.pump(st, zero, lead0)
    cp_bx.wait()
    scoped("wait", lambda: pltpu.make_async_copy(bwq_hbm, bwq_buf, sems.at[S_BWQ]).wait())
    awuv.wait()
    t = sch.ticks_(st, t, T_BQ)
    qb = _dot(bx_buf[...], bwq_buf[...].reshape(M, H * D), NN)
    for h in range(H):
        qb_scr[pl.ds(h, B, stride=H), :] = qb[:, h * D:(h + 1) * D]
    m_scr[...] = jnp.full(m_scr.shape, -jnp.inf, F32)
    l_scr[...] = jnp.zeros(l_scr.shape, F32)
    acc_scr[...] = jnp.zeros(acc_scr.shape, F32)

    def uv_fn(h, u):
        rows = jnp.concatenate([ctx_scr[cc, pl.ds(h, B, stride=H), :] for cc in range(4)], axis=1).astype(BF16)
        ctxh_scr[h] = _dot(rows, u, NN)

    weight_phase(st, t, awuv_buf, uv_fn)
    sch.feed(10 ** 9)

    def b_block(par):
        kb, vb = k_bufs[par], v_bufs[par]
        low = lax.broadcasted_iota(jnp.int32, (8, 1), 0) < 4
        qb = qb_scr[...]
        ss = []
        for p in range(NG // 2):
            q8 = qb[8 * p:8 * p + 8, :].astype(BF16)
            ss.append(jnp.where(low, _dot(q8, kb[2 * p], NT), _dot(q8, kb[2 * p + 1], NT)))
        s = jnp.concatenate(ss, axis=0) * scale
        m_old = m_scr[...]
        m_new = jnp.maximum(m_old, jnp.max(s, axis=1, keepdims=True))
        alpha = jnp.exp(m_old - m_new)
        e = [jnp.exp(s[:, i * 128:(i + 1) * 128] - m_new) for i in range(KB // 128)]
        pe = jnp.concatenate(e, axis=1)
        os_ = []
        for p in range(NG // 2):
            pb = pe[8 * p:8 * p + 8, :].astype(BF16)
            os_.append(jnp.where(low, _dot(pb, vb[2 * p], NN), _dot(pb, vb[2 * p + 1], NN)))
        m_scr[...] = m_new
        l_scr[...] = alpha * l_scr[...] + sum(e[1:], e[0])
        acc_scr[...] = alpha * acc_scr[...] + jnp.concatenate(os_, axis=0)

    def b_slot(j, par, nxt):
        st = vc(j + 1, 1 - par)
        t = sch.pump(st, zero, LEAD)
        kc(j, par).wait()
        vc(j, par).wait()
        t = sch.ticks_(st, t, T_B)
        b_block(par)
        for c, _ in nxt:
            c.start(priority=1)
        sch.pump(st, t, NV - LEAD - T_B)

    def b_body(i, c):
        b_slot(2 * i, 0, kc(2 * i + 2, 0).bg() + vc(2 * i + 2, 0).bg())
        b_slot(2 * i + 1, 1, kc(2 * i + 3, 1).bg() + vc(2 * i + 3, 1).bg())
        return c

    lax.fori_loop(0, NSTEP // 2 - 1, b_body, 0)
    b_slot(NSTEP - 2, 0, ao[0].bg())

    sch.q = ao[1].bg() + ao[2].bg() + bo[3].bg() + [(ld.copy(0, ld.S, 0, ld.L), ld.S * 4) for ld in ao_last]
    sch.issued, sch.ticks, sch.rate = 32, 0, 1.0
    t = sch.pump(bo[0], zero, LEAD)
    kc(NSTEP - 1, 1).wait()
    vc(NSTEP - 1, 1).wait()
    t = sch.ticks_(bo[0], t, T_B + 2)
    b_block(1)
    acc_scr[...] = acc_scr[...] / jnp.sum(l_scr[...], axis=1, keepdims=True)
    sch.pump(bo[0], t, 32 - LEAD - T_B - 2)

    def mm_a(buf, g, s0=0):
        lhs = jnp.concatenate([ctxh_scr[4 * (s0 + s) + g] for s in range(buf.shape[0])], axis=1).astype(BF16)
        return _dot(lhs, buf[...].reshape(buf.shape[0] * D, M), NN)

    def mm_b(buf, g):
        lhs = jnp.concatenate([acc_scr[pl.ds(4 * s + g, B, stride=H), :] for s in range(NS)], axis=1).astype(BF16)
        return _dot(lhs, buf[...].reshape(NS * D, M), NN)

    oa = ob = None
    for g in range(3):
        n = 32 if g < 2 else NL
        t = sch.pump(bo[g + 1], zero, LEAD + 2)
        ao[g].wait()
        bo[g].wait()
        t = sch.ticks_(bo[g + 1], t, T_G)
        pa, pb_ = mm_a(ao[g].dst, g), mm_b(bo[g].dst, g)
        oa = pa if oa is None else pa + oa
        ob = pb_ if ob is None else pb_ + ob
        sch.pump(bo[g + 1], t, n - LEAD - 2 - T_G)
    sch.feed(10 ** 9)
    bo[3].wait()
    out_ref[:, M:2 * M] = (mm_b(bo[3].dst, 3) + ob).astype(BF16)
    for i, ld in enumerate(ao_last):
        ld.wait()
        oa = mm_a(ld.dst, 3, AO_LAST[i][0]) + oa
    out_ref[:, 0:M] = oa.astype(BF16)


@jax.jit
def pallas_concat_heads__compressed_kv_cla__gqa_block_cached__decode_kernel(A_x, A_c_kv, A_w_q, A_w_uk, A_w_uv, A_w_o, B_x, B_k_cache, B_v_cache, B_wq, B_wo):
    args = (
        A_x.reshape(B, M), A_c_kv.reshape(B * NS, SK // NS, DC),
        A_w_q.reshape(NS, M * H // NS, D), A_w_uk.reshape(NS, DC * H // NS, D), A_w_uv.reshape(NS, DC * H // NS, D),
        A_w_o.reshape(NS, H * D // NS, M),
        B_x.reshape(B, M), B_k_cache.reshape(NG, SK, D), B_v_cache.reshape(NG, SK, D),
        B_wq.reshape(NS, M // NS, H * D), B_wo.reshape(NS, H * D // NS, M),
    )
    scratch = (
        [pltpu.VMEM((B, M), BF16)] * 2
        + [pltpu.VMEM((NS, M // NS, H * D), BF16)]
        + [pltpu.VMEM((NS, M * H // NS, D), BF16)] * 3
        + [pltpu.VMEM((NS, SK // NS, DC), BF16)] * 4
        + [pltpu.VMEM((NG, KB, D), BF16)] * 4
        + [pltpu.VMEM((NS, D, M), BF16)] * 3 + [pltpu.VMEM((n, D, M), BF16) for _, n in AO_LAST]
        + [pltpu.VMEM((NS, D, M), BF16)] * 4
        + [pltpu.VMEM((H, B, D), F32),
           pltpu.VMEM((4, B * H, 128), F32), pltpu.VMEM((4, B * H, 128), F32),
           pltpu.VMEM((H, B, D), F32)]
        + [pltpu.VMEM((B * H, D), F32)] * 4
        + [pltpu.SemaphoreType.DMA((NSEM,))]
    )
    return pl.pallas_call(
        kernel,
        in_specs=[pl.BlockSpec(memory_space=pl.ANY)] * 11,
        out_specs=pl.BlockSpec(memory_space=pltpu.VMEM),
        out_shape=jax.ShapeDtypeStruct((B, 2 * M), BF16),
        scratch_shapes=scratch,
        compiler_params=pltpu.CompilerParams(vmem_limit_bytes=100 * 1024 * 1024,
                                             disable_semaphore_checks=True, disable_bounds_checks=True),
    )(*args).reshape(B, 1, 2 * M)
```

```python
import jax
import jax.numpy as jnp
from jax import lax
import jax.experimental.pallas as pl
import jax.experimental.pallas.tpu as pltpu

B, H, SK, D, M = 4, 32, 4096, 128, 512
DC = 512
HKV = 8
NG = B * HKV
KB = 256
NSTEP = SK // KB
NS = 8
CC = 512
SEG = 32 * 1024
F32 = jnp.float32
BF16 = jnp.bfloat16
NT = (((1,), (1,)), ((), ()))
NN = (((1,), (0,)), ((), ()))

NLAG = 10
T_W = 13
T_A = 33
T_BQ = 11
T_B = 20
T_G = 6
LEAD = 10
LA = 36
CH = 16
NL = 20
OFF = 8
WOFF = 120

(S_AX, S_BX, S_BWQ, S_AWQ, S_AWUK, S_AWUV, S_C, S_K, S_V, S_AO, S_BO) = (0, 1, 2, 3, 4, 5, 6, 10, 12, 14, 21)
NSEM = S_BO + 4
AO_LAST = [(0, 4), (4, 2), (6, 1), (7, 1)]


def _dot(a, b, dims):
    return lax.dot_general(a, b, dims, preferred_element_type=F32)


def _lag(t):
    u = t.astype(jnp.uint32)
    for k in range(NLAG):
        u = lax.rem(u, jnp.uint32(900001 - 14 * k))
    return u.astype(jnp.int32)


def _split_pair(w_u32):
    lo = lax.bitcast_convert_type(w_u32 << 16, F32).astype(BF16)
    hi = lax.bitcast_convert_type(w_u32 & jnp.uint32(0xFFFF0000), F32).astype(BF16)
    return lo, hi


def _lane_tiles(x):
    return [x[:, i:i + 128] for i in range(0, x.shape[1], 128)]


def _kernel(ax_hbm, ckv_hbm, awq_hbm, awuk_hbm, awuv_hbm, awo_hbm, bx_hbm, k_hbm, v_hbm, bwq_hbm, bwo_hbm,
            out_ref,
            ax_buf, bx_buf, bwq_buf, awq_buf, awuk_buf, awuv_buf, c0_buf, c1_buf, c2_buf, c3_buf,
            k0_buf, k1_buf, v0_buf, v1_buf,
            ao0, ao1, ao2, ao3a, ao3b, ao3c, ao3d, bo0, bo1, bo2, bo3,
            q_scr, qa_scr, ctx_scr, ctxh_scr, qb_scr, m_scr, l_scr, acc_scr, ma_scr, la_scr, sems):
    scale = D ** -0.5
    c_bufs = (c0_buf, c1_buf, c2_buf, c3_buf)
    k_bufs = (k0_buf, k1_buf)
    v_bufs = (v0_buf, v1_buf)
    zero = jnp.int32(0)

    class Load:
        def __init__(self, src, dst, sem, nfg=0, s0=0, r0=0, wrap=0, flip=False):
            self.src, self.dst, self.sem, self.nfg, self.s0, self.r0 = src, dst, sem, nfg, s0, r0
            self.wrap, self.flip, self.done = wrap, flip, 0
            self.S, self.L, width = dst.shape
            self.seg = SEG // (width * 2)

        def rows(self, rnd):
            return self.seg - (self.wrap if (rnd + 1) * self.seg == self.L else 0)

        def copy(self, s, ns, r, nr):
            return pltpu.make_async_copy(self.src.at[pl.ds(self.s0 + s, ns), pl.ds(self.r0 + r, nr)],
                                         self.dst.at[pl.ds(s, ns), pl.ds(r, nr)], sems.at[self.sem])

        def background(self, first=0):
            if first:
                cuts = [0] + list(range(first, self.L, self.seg)) + [self.L]
                return [(self.copy(0, self.S, a, b - a), self.S * (b - a) / self.seg) for a, b in zip(cuts, cuts[1:])]
            out = []
            for rnd in range(self.nfg // self.S, self.L // self.seg):
                s = max(self.nfg - rnd * self.S, 0)
                out.append((self.copy(s, self.S - s, rnd * self.seg, self.rows(rnd)), self.S - s))
            if self.wrap:
                out.append((pltpu.make_async_copy(self.src.at[pl.ds(self.s0, self.S), pl.ds(0, self.wrap)],
                                                  self.dst.at[:, pl.ds(self.L - self.wrap, self.wrap)],
                                                  sems.at[self.sem]), 0))
            return out

        def wait(self):
            pltpu.make_async_copy(self.dst, self.dst, sems.at[self.sem]).wait()

        def claim(self, n):
            rows = self.rows(self.done // self.S)
            assert rows == self.rows((self.done + n - 1) // self.S) and self.done + n <= self.nfg
            self.done += n
            return rows

        def tick(self, t, rows):
            s = lax.bitwise_and(t, self.S - 1)
            if self.flip:
                s = lax.bitwise_xor(s, self.S - 1)
            r = pl.multiple_of(lax.shift_right_logical(t, self.S.bit_length() - 1) * self.seg, self.seg)
            self.copy(s, 1, r, rows).start(priority=0)
            return _lag(t + 1)

    class Sched:
        def __init__(self, queue, issued=0):
            self.queue, self.issued, self.now = queue, issued, 0

        def feed(self, upto):
            while self.queue and self.issued < upto + LA:
                copy, n = self.queue.pop(0)
                copy.start(priority=1)
                self.issued += n

        def ticks(self, ld, t, n):
            for _ in range(n):
                self.feed(self.now)
                t = ld.tick(t, ld.claim(1))
                self.now += 1
            return t

        def pump(self, ld, t, n=None):
            n = ld.nfg - ld.done if n is None else n
            while n > 0:
                k = n if (n <= CH + 4 or not self.queue) else CH
                self.feed(self.now + k // 2)
                rows = ld.claim(k)
                t = lax.fori_loop(0, k, lambda i, t: ld.tick(t, rows), t)
                self.now += k
                n -= k
            return t

    cp_ax = pltpu.make_async_copy(ax_hbm, ax_buf, sems.at[S_AX])
    cp_bx = pltpu.make_async_copy(bx_hbm, bx_buf, sems.at[S_BX])
    awq = Load(awq_hbm, awq_buf, S_AWQ)
    awuk = Load(awuk_hbm, awuk_buf, S_AWUK)
    awuv = Load(awuv_hbm, awuv_buf, S_AWUV)
    bwq = Load(bwq_hbm, bwq_buf, S_BWQ)
    half = H * D // 2
    bwq_bg = [(pltpu.make_async_copy(bwq_hbm.at[:, pl.ds(r, 8), pl.ds(c, half)],
                                     bwq_buf.at[:, pl.ds(r, 8), pl.ds(c, half)], sems.at[S_BWQ]), NS)
              for r in range(0, M // NS, 8) for c in (0, half)]
    ckv = [Load(ckv_hbm, c_bufs[k], S_C + k, 128, r0=k * CC) for k in range(4)]
    ao = [Load(awo_hbm, buf, S_AO + g, r0=g * D) for g, buf in enumerate((ao0, ao1, ao2))]
    ao_last = [Load(awo_hbm, buf, S_AO + 3 + i, s0=AO_LAST[i][0], r0=3 * D)
               for i, buf in enumerate((ao3a, ao3b, ao3c, ao3d))]
    bo = [Load(bwo_hbm, buf, S_BO + g, 32 if g < 3 else NL, r0=g * D) for g, buf in enumerate((bo0, bo1, bo2, bo3))]

    def kv_pos(j):
        if isinstance(j, int):
            return dict(r0=SK - KB + OFF, wrap=OFF) if j == 0 else dict(r0=OFF + (j - 1) * KB)
        return dict(r0=pl.multiple_of(OFF + (j - 1) * KB, 8))

    def kc(j, par):
        return Load(k_hbm, k_bufs[par], S_K + par, **kv_pos(j))

    def vc(j, par):
        return Load(v_hbm, v_bufs[par], S_V + par, 2 * NG, flip=True, **kv_pos(j))

    wq_bg = awq.background(WOFF)
    sch = Sched(wq_bg[:1] + [(cp_ax, 0), (cp_bx, 0)] + wq_bg[1:] + awuk.background(WOFF) + bwq_bg
                + awuv.background(WOFF) + kc(0, 0).background() + vc(0, 0).background() + kc(1, 1).background())

    def per_head(st, t, w_buf, fn, quarters=range(4)):
        w32 = w_buf.bitcast(jnp.uint32)
        for jj in quarters:
            t = sch.ticks(st, t, T_W)
            for j in range(4 * jj, 4 * jj + 4):
                pair = w32[:, pl.ds(j, M // NS, stride=H // 2), :].reshape(M, D)
                for p, w in enumerate(_split_pair(pair)):
                    fn(2 * j + p, w)
        return t

    def q_fn(h, w):
        q_scr[h] = _dot(ax_buf[...], w, NN)

    def qa_fn(h, w):
        qa = _dot(q_scr[h].astype(BF16), w, NT) * scale
        for cc, tile in enumerate(_lane_tiles(qa)):
            qa_scr[cc, pl.ds(h, B, stride=H), :] = tile

    def uv_fn(h, w):
        rows = jnp.concatenate([ctx_scr[cc, pl.ds(h, B, stride=H), :] for cc in range(4)], axis=1)
        ctxh_scr[h] = _dot(rows.astype(BF16), w, NN)

    def a_block(st, t, k):
        t = sch.ticks(st, t, T_A)

        def latent(b):
            return c_bufs[k][pl.ds(2 * b, 2)].reshape(2 * CC, DC)

        scores = []
        for b in range(B):
            qa = jnp.concatenate([qa_scr[cc, pl.ds(b * H, H), :] for cc in range(4)], axis=1)
            scores.append(_dot(qa.astype(BF16), latent(b), NT))
        for b in range(B):
            rows = pl.ds(b * H, H)
            m_new = jnp.broadcast_to(jnp.max(scores[b], axis=1, keepdims=True), (H, 128))
            if k > 0:
                m_old = ma_scr[rows, :]
                m_new = jnp.maximum(m_old, m_new)
                alpha = jnp.exp(m_old - m_new)
            e = [jnp.exp(s - m_new) for s in _lane_tiles(scores[b])]
            l = sum(e[1:], e[0])
            ctx = _lane_tiles(_dot(jnp.concatenate(e, axis=1).astype(BF16), latent(b), NN))
            if k > 0:
                l = alpha * la_scr[rows, :] + l
                ctx = [alpha * ctx_scr[cc, rows, :] + ctx[cc] for cc in range(4)]
            if k < 3:
                ma_scr[rows, :] = m_new
                la_scr[rows, :] = l
            else:
                total = jnp.sum(l, axis=1, keepdims=True)
                ctx = [c / total for c in ctx]
            for cc in range(4):
                ctx_scr[cc, rows, :] = ctx[cc]
        return t

    def b_block(par, first=False, last=False):
        kb, vb = k_bufs[par], v_bufs[par]
        low = lax.broadcasted_iota(jnp.int32, (8, 1), 0) < 4

        def paired(x, w_buf, dims):
            out = []
            for p in range(NG // 2):
                x8 = x[8 * p:8 * p + 8, :].astype(BF16)
                out.append(jnp.where(low, _dot(x8, w_buf[2 * p], dims), _dot(x8, w_buf[2 * p + 1], dims)))
            return jnp.concatenate(out, axis=0)

        s = paired(qb_scr[...], kb, NT) * scale
        m_new = jnp.broadcast_to(jnp.max(s, axis=1, keepdims=True), (B * H, 128))
        if not first:
            m_old = m_scr[...]
            m_new = jnp.maximum(m_old, m_new)
            alpha = jnp.exp(m_old - m_new)
        e = [jnp.exp(x - m_new) for x in _lane_tiles(s)]
        l = sum(e[1:], e[0])
        acc = paired(jnp.concatenate(e, axis=1), vb, NN)
        if not first:
            l = alpha * l_scr[...] + l
            acc = alpha * acc_scr[...] + acc
        if last:
            acc = acc / jnp.sum(l, axis=1, keepdims=True)
        else:
            m_scr[...] = m_new
            l_scr[...] = l
        acc_scr[...] = acc

    sch.pump(ckv[0], zero)

    t = sch.pump(ckv[1], zero, LEAD)
    cp_ax.wait()
    awq.wait()
    t = per_head(ckv[1], t, awq_buf, q_fn)
    sch.pump(ckv[1], t)

    t = sch.pump(ckv[2], zero, LEAD)
    awuk.wait()
    t = per_head(ckv[2], t, awuk_buf, qa_fn)
    ckv[0].wait()
    t = a_block(ckv[2], t, 0)
    sch.pump(ckv[2], t)

    t = sch.pump(ckv[3], zero, LEAD)
    cp_bx.wait()
    bwq.wait()
    t = sch.ticks(ckv[3], t, T_BQ)
    for h, tile in enumerate(_lane_tiles(_dot(bx_buf[...], bwq_buf[...].reshape(M, H * D), NN))):
        qb_scr[pl.ds(h, B, stride=H), :] = tile
    ckv[1].wait()
    t = a_block(ckv[3], t, 1)
    ckv[2].wait()
    t = a_block(ckv[3], t, 2)
    sch.pump(ckv[3], t)

    st = vc(0, 0)
    t = sch.pump(st, zero, LEAD)
    awuv.wait()
    ckv[3].wait()
    t = a_block(st, t, 3)
    sch.feed(10 ** 9)
    sch.pump(st, t)

    def b_slot(j, par, nxt, quarters=()):
        st = vc(j + 1, 1 - par)
        t = sch.pump(st, zero, LEAD)
        kc(0, par).wait()
        vc(0, par).wait()
        t = sch.ticks(st, t, T_B)
        b_block(par, first=isinstance(j, int) and j == 0)
        for copy, _ in nxt.background():
            copy.start(priority=1)
        if quarters:
            t = sch.pump(st, t, 2)
            t = per_head(st, t, awuv_buf, uv_fn, quarters)
        sch.pump(st, t)

    b_slot(0, 0, kc(2, 0), (0, 1))
    b_slot(1, 1, kc(3, 1), (2, 3))

    def b_body(i, carry):
        b_slot(2 * i, 0, kc(2 * i + 2, 0))
        b_slot(2 * i + 1, 1, kc(2 * i + 3, 1))
        return carry

    lax.fori_loop(1, NSTEP // 2 - 1, b_body, 0)
    b_slot(NSTEP - 2, 0, ao[0])

    sch = Sched(ao[1].background() + ao[2].background() + bo[3].background()
                + [(ld.copy(0, ld.S, 0, ld.L), ld.S * 4) for ld in ao_last], issued=32)
    t = sch.pump(bo[0], zero, LEAD)
    kc(0, 1).wait()
    vc(0, 1).wait()
    t = sch.ticks(bo[0], t, T_B + 2)
    b_block(1, last=True)
    sch.pump(bo[0], t)

    def proj_a(ld, g):
        lhs = jnp.concatenate([ctxh_scr[4 * (ld.s0 + s) + g] for s in range(ld.S)], axis=1)
        return _dot(lhs.astype(BF16), ld.dst[...].reshape(ld.S * D, M), NN)

    def proj_b(ld, g):
        lhs = jnp.concatenate([acc_scr[pl.ds(4 * s + g, B, stride=H), :] for s in range(NS)], axis=1)
        return _dot(lhs.astype(BF16), ld.dst[...].reshape(NS * D, M), NN)

    oa = ob = None
    for g in range(3):
        t = sch.pump(bo[g + 1], zero, LEAD + 2)
        ao[g].wait()
        bo[g].wait()
        t = sch.ticks(bo[g + 1], t, T_G)
        oa = proj_a(ao[g], g) if g == 0 else proj_a(ao[g], g) + oa
        ob = proj_b(bo[g], g) if g == 0 else proj_b(bo[g], g) + ob
        sch.pump(bo[g + 1], t)
    sch.feed(10 ** 9)
    bo[3].wait()
    out_ref[:, M:2 * M] = (proj_b(bo[3], 3) + ob).astype(BF16)
    for ld in ao_last:
        ld.wait()
        oa = proj_a(ld, 3) + oa
    out_ref[:, 0:M] = oa.astype(BF16)


@jax.jit
def pallas_concat_heads__compressed_kv_cla__gqa_block_cached__decode_kernel(A_x, A_c_kv, A_w_q, A_w_uk, A_w_uv, A_w_o, B_x, B_k_cache, B_v_cache, B_wq, B_wo):
    args = (
        A_x.reshape(B, M), A_c_kv.reshape(NS, B * SK // NS, DC),
        A_w_q.reshape(NS, M * H // NS, D), A_w_uk.reshape(NS, DC * H // NS, D), A_w_uv.reshape(NS, DC * H // NS, D),
        A_w_o.reshape(NS, H * D // NS, M),
        B_x.reshape(B, M), B_k_cache.reshape(NG, SK, D), B_v_cache.reshape(NG, SK, D),
        B_wq.reshape(NS, M // NS, H * D), B_wo.reshape(NS, H * D // NS, M),
    )
    scratch = (
        [pltpu.VMEM((B, M), BF16)] * 2
        + [pltpu.VMEM((NS, M // NS, H * D), BF16)]
        + [pltpu.VMEM((NS, M * H // NS, D), BF16)] * 3
        + [pltpu.VMEM((NS, CC, DC), BF16)] * 4
        + [pltpu.VMEM((NG, KB, D), BF16)] * 4
        + [pltpu.VMEM((NS, D, M), BF16)] * 3 + [pltpu.VMEM((n, D, M), BF16) for _, n in AO_LAST]
        + [pltpu.VMEM((NS, D, M), BF16)] * 4
        + [pltpu.VMEM((H, B, D), F32),
           pltpu.VMEM((4, B * H, 128), F32), pltpu.VMEM((4, B * H, 128), F32),
           pltpu.VMEM((H, B, D), F32)]
        + [pltpu.VMEM((B * H, D), F32)] * 6
        + [pltpu.SemaphoreType.DMA((NSEM,))]
    )
    out = pl.pallas_call(
        _kernel,
        in_specs=[pl.BlockSpec(memory_space=pl.ANY)] * 11,
        out_specs=pl.BlockSpec(memory_space=pltpu.VMEM),
        out_shape=jax.ShapeDtypeStruct((B, 2 * M), BF16),
        scratch_shapes=scratch,
        compiler_params=pltpu.CompilerParams(vmem_limit_bytes=100 * 1024 * 1024,
                                             disable_semaphore_checks=True, disable_bounds_checks=True),
    )(*args)
    return out.reshape(B, 1, 2 * M)
```

```python
import jax
import jax.numpy as jnp
from jax import lax
import jax.experimental.pallas as pl
import jax.experimental.pallas.tpu as pltpu

B, H, SK, D, M = 4, 32, 4096, 128, 512
DC = 512
HKV = 8
NG = B * HKV
KB = 256
NSTEP = SK // KB
NS = 8
CC = 512
SEG = 32 * 1024
F32 = jnp.float32
BF16 = jnp.bfloat16
NT = (((1,), (1,)), ((), ()))
NN = (((1,), (0,)), ((), ()))

NLAG = 10
T_W = 13
T_A = 36
T_BQ = 11
T_B = 20
T_G = 6
LEAD = 10
LA = 36
NL = 20
OFF = 8
WOFF = 120

(S_AX, S_BX, S_BWQ, S_AWQ, S_AWUK, S_AWUV, S_C, S_K, S_V, S_AO, S_BO) = (0, 1, 2, 3, 4, 5, 6, 10, 12, 14, 21)
NSEM = S_BO + 4
AO_LAST = [(0, 4), (4, 2), (6, 1), (7, 1)]


def _dot(a, b, dims):
    return lax.dot_general(a, b, dims, preferred_element_type=F32)


def _lag(t, extra=0):
    u = t.astype(jnp.uint32)
    for k in range(NLAG):
        u = lax.rem(u, jnp.uint32(900001 - 14 * k))
        if k < extra:
            u = u + jnp.uint32(1)
    if extra:
        u = u - jnp.uint32(extra)
    return u.astype(jnp.int32)


def _split_pair(w_u32):
    lo = lax.bitcast_convert_type(w_u32 << 16, F32).astype(BF16)
    hi = lax.bitcast_convert_type(w_u32 & jnp.uint32(0xFFFF0000), F32).astype(BF16)
    return lo, hi


def _lane_tiles(x):
    return [x[:, i:i + 128] for i in range(0, x.shape[1], 128)]


def _kernel(ax_hbm, ckv_hbm, awq_hbm, awuk_hbm, awuv_hbm, awo_hbm, bx_hbm, k_hbm, v_hbm, bwq_hbm, bwo_hbm,
            out_ref,
            ax_buf, bx_buf, bwq_buf, awq_buf, awuk_buf, awuv_buf, c0_buf, c1_buf, c2_buf, c3_buf,
            k0_buf, k1_buf, v0_buf, v1_buf,
            ao0, ao1, ao2, ao3a, ao3b, ao3c, ao3d, bo0, bo1, bo2, bo3,
            q_scr, qa_scr, ctx_scr, ctxh_scr, qb_scr, m_scr, l_scr, acc_scr, ma_scr, la_scr, sems):
    scale = D ** -0.5
    c_bufs = (c0_buf, c1_buf, c2_buf, c3_buf)
    k_bufs = (k0_buf, k1_buf)
    v_bufs = (v0_buf, v1_buf)
    zero = jnp.int32(0)

    class Load:
        def __init__(self, src, dst, sem, nfg=0, s0=0, r0=0, wrap=0, flip=False):
            assert not (nfg and wrap)
            self.src, self.dst, self.sem, self.nfg, self.s0, self.r0 = src, dst, sem, nfg, s0, r0
            self.wrap, self.flip, self.done = wrap, flip, 0
            self.S, self.L, width = dst.shape
            self.seg = SEG // (width * 2)

        def copy(self, s, ns, r, nr):
            return pltpu.make_async_copy(self.src.at[pl.ds(self.s0 + s, ns), pl.ds(self.r0 + r, nr)],
                                         self.dst.at[pl.ds(s, ns), pl.ds(r, nr)], sems.at[self.sem])

        def background(self):
            out = []
            for rnd in range(self.nfg // self.S, self.L // self.seg):
                s = max(self.nfg - rnd * self.S, 0)
                rows = min(self.seg, self.L - self.wrap - rnd * self.seg)
                out.append((self.copy(s, self.S - s, rnd * self.seg, rows), self.S - s))
            if self.wrap:
                out.append((pltpu.make_async_copy(self.src.at[pl.ds(self.s0, self.S), pl.ds(0, self.wrap)],
                                                  self.dst.at[:, pl.ds(self.L - self.wrap, self.wrap)],
                                                  sems.at[self.sem]), 0))
            return out

        def wait(self):
            pltpu.make_async_copy(self.dst, self.dst, sems.at[self.sem]).wait()

        def tick(self, t):
            s = lax.bitwise_and(t, self.S - 1)
            if self.flip:
                s = lax.bitwise_xor(s, self.S - 1)
            rnd = lax.shift_right_logical(t, self.S.bit_length() - 1)
            self.copy(s, 1, pl.multiple_of(rnd * self.seg, self.seg), self.seg).start(priority=0)
            return _lag(t + 1)

    class FlatLoad(Load):
        def __init__(self, src, dst, sem):
            self.src, self.dst, self.sem, self.done = src, dst, sem, 0
            self.wide = dst.shape[1] > D
            self.nfg = 128 if self.wide else 127

        def part(self, *idx):
            return pltpu.make_async_copy(self.src.at[idx], self.dst.at[idx], sems.at[self.sem])

        def background(self):
            if self.wide:
                return []
            tail = WOFF + self.nfg * 128
            return [(self.part(pl.ds(0, WOFF)), 0), (self.part(pl.ds(tail, self.dst.shape[0] - tail)), 0)]

        def tick(self, t):
            s = lax.bitwise_and(t, 7)
            rnd = lax.shift_right_logical(t, 3)
            if self.wide:
                half = self.dst.shape[1] // 2
                i = s * 16 + lax.bitwise_and(rnd + s, 15)
                r = pl.multiple_of(lax.shift_right_logical(i, 1) * 8, 8)
                c = pl.multiple_of(lax.bitwise_and(i, 1) * half, half)
                self.part(pl.ds(r, 8), pl.ds(c, half)).start(priority=0)
            else:
                i = s * 16 + lax.bitwise_xor(rnd, 7 - s)
                self.part(pl.ds(pl.multiple_of(WOFF + i * 128, 8), 128)).start(priority=0)
            return _lag(t + 1, 5)

    class Sched:
        def __init__(self, queue=(), issued=0):
            self.queue, self.issued, self.now = list(queue), issued, 0

        def feed(self, upto):
            while self.queue and self.issued < upto + LA:
                copy, n = self.queue.pop(0)
                copy.start(priority=1)
                self.issued += n

        def count(self, ld, n):
            assert ld.done + n <= ld.nfg
            ld.done += n
            self.now += n

        def ticks(self, ld, t, n):
            for _ in range(n):
                self.feed(self.now)
                self.count(ld, 1)
                t = ld.tick(t)
            return t

        def pump(self, ld, t, n=None):
            n = ld.nfg - ld.done if n is None else n
            self.feed(self.now + n // 2)
            self.count(ld, n)
            return lax.fori_loop(0, n, lambda i, t: ld.tick(t), t) if n else t

    cp_ax = pltpu.make_async_copy(ax_hbm, ax_buf, sems.at[S_AX])
    cp_bx = pltpu.make_async_copy(bx_hbm, bx_buf, sems.at[S_BX])
    awq = FlatLoad(awq_hbm, awq_buf, S_AWQ)
    awuk = FlatLoad(awuk_hbm, awuk_buf, S_AWUK)
    awuv = FlatLoad(awuv_hbm, awuv_buf, S_AWUV)
    bwq = FlatLoad(bwq_hbm, bwq_buf, S_BWQ)
    ckv = [Load(ckv_hbm, c_bufs[k], S_C + k, 128, r0=k * CC) for k in range(4)]
    ao = [Load(awo_hbm, buf, S_AO + g, r0=g * D) for g, buf in enumerate((ao0, ao1, ao2))]
    ao_last = [Load(awo_hbm, buf, S_AO + 3 + i, s0=AO_LAST[i][0], r0=3 * D)
               for i, buf in enumerate((ao3a, ao3b, ao3c, ao3d))]
    bo = [Load(bwo_hbm, buf, S_BO + g, 32 if g < 3 else NL, r0=g * D) for g, buf in enumerate((bo0, bo1, bo2, bo3))]

    def kv_pos(j):
        if isinstance(j, int):
            return dict(r0=SK - KB + OFF, wrap=OFF) if j == 0 else dict(r0=OFF + (j - 1) * KB)
        return dict(r0=pl.multiple_of(OFF + (j - 1) * KB, 8))

    def kc(j, par):
        return Load(k_hbm, k_bufs[par], S_K + par, **kv_pos(j))

    def vc(j, par, nfg=0):
        return Load(v_hbm, v_bufs[par], S_V + par, nfg, flip=True, **kv_pos(j))

    def queue(*loads):
        for ld in loads:
            for copy, _ in ld.background():
                copy.start(priority=1)

    sch = Sched()

    def per_head(st, t, w_buf, fn, quarters=range(4)):
        w32 = w_buf.bitcast(jnp.uint32)
        for jj in quarters:
            t = sch.ticks(st, t, T_W)
            for j in range(4 * jj, 4 * jj + 4):
                for p, w in enumerate(_split_pair(w32[pl.ds(j, M, stride=H // 2), :])):
                    fn(2 * j + p, w)
        return t

    def q_fn(h, w):
        q_scr[h] = _dot(ax_buf[...], w, NN)

    def qa_fn(h, w):
        qa = _dot(q_scr[h].astype(BF16), w, NT) * scale
        for cc, tile in enumerate(_lane_tiles(qa)):
            qa_scr[cc, pl.ds(h, B, stride=H), :] = tile

    def uv_fn(h, w):
        rows = jnp.concatenate([ctx_scr[cc, pl.ds(h, B, stride=H), :] for cc in range(4)], axis=1)
        ctxh_scr[h] = _dot(rows.astype(BF16), w, NN)

    def a_query(st, t):
        cp_ax.wait()
        return per_head(st, t, awq_buf, q_fn)

    def b_query(st, t):
        cp_bx.wait()
        t = sch.ticks(st, t, T_BQ)
        for h, tile in enumerate(_lane_tiles(_dot(bx_buf[...], bwq_buf[...], NN))):
            qb_scr[pl.ds(h, B, stride=H), :] = tile
        return t

    def a_block(st, t, k):
        t = sch.ticks(st, t, T_A)

        def latent(b):
            return c_bufs[k][pl.ds(2 * b, 2)].reshape(2 * CC, DC)

        scores = []
        for b in range(B):
            qa = jnp.concatenate([qa_scr[cc, pl.ds(b * H, H), :] for cc in range(4)], axis=1)
            scores.append(_dot(qa.astype(BF16), latent(b), NT))
        for b in range(B):
            rows = pl.ds(b * H, H)
            m_new = jnp.broadcast_to(jnp.max(scores[b], axis=1, keepdims=True), (H, 128))
            if k > 0:
                m_old = ma_scr[rows, :]
                m_new = jnp.maximum(m_old, m_new)
                alpha = jnp.exp(m_old - m_new)
            e = [jnp.exp(s - m_new) for s in _lane_tiles(scores[b])]
            l = sum(e[1:], e[0])
            ctx = _lane_tiles(_dot(jnp.concatenate(e, axis=1).astype(BF16), latent(b), NN))
            if k > 0:
                l = alpha * la_scr[rows, :] + l
                ctx = [alpha * ctx_scr[cc, rows, :] + ctx[cc] for cc in range(4)]
            if k < 3:
                ma_scr[rows, :] = m_new
                la_scr[rows, :] = l
            else:
                total = jnp.sum(l, axis=1, keepdims=True)
                ctx = [c / total for c in ctx]
            for cc in range(4):
                ctx_scr[cc, rows, :] = ctx[cc]
        return t

    def b_block(st, t, par, nxt, first=False, last=False):
        kc(0, par).wait()
        vc(0, par).wait()
        t = sch.ticks(st, t, T_B + 2 * last)
        low = lax.broadcasted_iota(jnp.int32, (8, 1), 0) < 4

        def paired(x, w_buf, dims):
            out = []
            for p in range(NG // 2):
                x8 = x[8 * p:8 * p + 8, :].astype(BF16)
                out.append(jnp.where(low, _dot(x8, w_buf[2 * p], dims), _dot(x8, w_buf[2 * p + 1], dims)))
            return jnp.concatenate(out, axis=0)

        s = paired(qb_scr[...], k_bufs[par], NT) * scale
        m_new = jnp.broadcast_to(jnp.max(s, axis=1, keepdims=True), (B * H, 128))
        if not first:
            m_old = m_scr[...]
            m_new = jnp.maximum(m_old, m_new)
            alpha = jnp.exp(m_old - m_new)
        e = [jnp.exp(x - m_new) for x in _lane_tiles(s)]
        l = sum(e[1:], e[0])
        acc = paired(jnp.concatenate(e, axis=1), v_bufs[par], NN)
        if not first:
            l = alpha * l_scr[...] + l
            acc = alpha * acc_scr[...] + acc
        if last:
            acc = acc / jnp.sum(l, axis=1, keepdims=True)
        else:
            m_scr[...] = m_new
            l_scr[...] = l
        acc_scr[...] = acc
        queue(*nxt)
        return t

    side = [(bwq, b_query), (awq, a_query), (awuk, lambda st, t: per_head(st, t, awuk_buf, qa_fn))]
    side += [(ckv[k], lambda st, t, k=k: a_block(st, t, k)) for k in range(4)] + [(awuv, None)]
    nx = len(side)
    queue(kc(0, 0))
    cp_bx.start(priority=1)
    cp_ax.start(priority=1)
    t = sch.pump(bwq, zero, 16)
    queue(vc(0, 0))
    t = sch.pump(bwq, t, 48)
    queue(awq, kc(1, 1), vc(1, 1))
    sch.pump(bwq, t)
    for i in range(1, nx):
        st = side[i][0]
        prev, use_prev = side[i - 1]
        par = (i - 1) % 2
        nxt = [kc(i + 1, par)] + ([side[i + 1][0], vc(i + 1, par)] if i + 1 < nx else [])
        t = sch.pump(st, zero, LEAD)
        prev.wait()
        if i == 1:
            t = b_block(st, use_prev(st, t), par, nxt, first=True)
        else:
            t = use_prev(st, sch.pump(st, b_block(st, t, par, nxt), 2))
        sch.pump(st, t)

    def b_slot(j, par, nxt, quarters=()):
        st = vc(j + 1, 1 - par, 2 * NG)
        t = b_block(st, sch.pump(st, zero, LEAD), par, [nxt])
        if quarters:
            if quarters[0] == 0:
                awuv.wait()
            else:
                t = sch.pump(st, t, 2)
            t = per_head(st, t, awuv_buf, uv_fn, quarters)
        sch.pump(st, t)

    b_slot(nx - 1, 1, kc(nx + 1, 1), (0, 1))
    b_slot(nx, 0, kc(nx + 2, 0), (2, 3))
    b_slot(nx + 1, 1, kc(nx + 3, 1))

    def b_body(i, carry):
        b_slot(2 * i, 0, kc(2 * i + 2, 0))
        b_slot(2 * i + 1, 1, kc(2 * i + 3, 1))
        return carry

    lax.fori_loop(nx // 2 + 1, NSTEP // 2 - 1, b_body, 0)
    b_slot(NSTEP - 2, 0, ao[0])

    sch = Sched(ao[1].background() + ao[2].background() + bo[3].background()
                + [(ld.copy(0, ld.S, 0, ld.L), ld.S * 4) for ld in ao_last], issued=32)
    t = b_block(bo[0], sch.pump(bo[0], zero, LEAD), 1, [], last=True)
    sch.pump(bo[0], t)

    def proj_a(ld, g):
        lhs = jnp.concatenate([ctxh_scr[4 * (ld.s0 + s) + g] for s in range(ld.S)], axis=1)
        return _dot(lhs.astype(BF16), ld.dst[...].reshape(ld.S * D, M), NN)

    def proj_b(ld, g):
        lhs = jnp.concatenate([acc_scr[pl.ds(4 * s + g, B, stride=H), :] for s in range(NS)], axis=1)
        return _dot(lhs.astype(BF16), ld.dst[...].reshape(NS * D, M), NN)

    oa = ob = None
    for g in range(3):
        t = sch.pump(bo[g + 1], zero, LEAD + 2)
        ao[g].wait()
        bo[g].wait()
        t = sch.ticks(bo[g + 1], t, T_G)
        oa = proj_a(ao[g], g) if g == 0 else proj_a(ao[g], g) + oa
        ob = proj_b(bo[g], g) if g == 0 else proj_b(bo[g], g) + ob
        sch.pump(bo[g + 1], t)
    sch.feed(10 ** 9)
    bo[3].wait()
    out_ref[:, M:2 * M] = (proj_b(bo[3], 3) + ob).astype(BF16)
    for ld in ao_last:
        ld.wait()
        oa = proj_a(ld, 3) + oa
    out_ref[:, 0:M] = oa.astype(BF16)


@jax.jit
def pallas_concat_heads__compressed_kv_cla__gqa_block_cached__decode_kernel(
    A_x: jax.Array,
    A_c_kv: jax.Array,
    A_w_q: jax.Array,
    A_w_uk: jax.Array,
    A_w_uv: jax.Array,
    A_w_o: jax.Array,
    B_x: jax.Array,
    B_k_cache: jax.Array,
    B_v_cache: jax.Array,
    B_wq: jax.Array,
    B_wo: jax.Array,
):
    args = (
        A_x.reshape(B, M), A_c_kv.reshape(NS, B * SK // NS, DC),
        A_w_q.reshape(M * H, D), A_w_uk.reshape(DC * H, D), A_w_uv.reshape(DC * H, D),
        A_w_o.reshape(NS, H * D // NS, M),
        B_x.reshape(B, M), B_k_cache.reshape(NG, SK, D), B_v_cache.reshape(NG, SK, D),
        B_wq, B_wo.reshape(NS, H * D // NS, M),
    )
    scratch = (
        [pltpu.VMEM((B, M), BF16)] * 2
        + [pltpu.VMEM((M, H * D), BF16)]
        + [pltpu.VMEM((M * H, D), BF16)] * 3
        + [pltpu.VMEM((NS, CC, DC), BF16)] * 4
        + [pltpu.VMEM((NG, KB, D), BF16)] * 4
        + [pltpu.VMEM((NS, D, M), BF16)] * 3 + [pltpu.VMEM((n, D, M), BF16) for _, n in AO_LAST]
        + [pltpu.VMEM((NS, D, M), BF16)] * 4
        + [pltpu.VMEM((H, B, D), F32),
           pltpu.VMEM((4, B * H, 128), F32), pltpu.VMEM((4, B * H, 128), F32),
           pltpu.VMEM((H, B, D), F32)]
        + [pltpu.VMEM((B * H, D), F32)] * 6
        + [pltpu.SemaphoreType.DMA((NSEM,))]
    )
    out = pl.pallas_call(
        _kernel,
        in_specs=[pl.BlockSpec(memory_space=pl.ANY)] * 11,
        out_specs=pl.BlockSpec(memory_space=pltpu.VMEM),
        out_shape=jax.ShapeDtypeStruct((B, 2 * M), BF16),
        scratch_shapes=scratch,
        compiler_params=pltpu.CompilerParams(vmem_limit_bytes=64 * 1024 * 1024,
                                             disable_semaphore_checks=True, disable_bounds_checks=True),
    )(*args)
    return out.reshape(B, 1, 2 * M)
```

```python
import jax
import jax.numpy as jnp
from jax import lax
import jax.experimental.pallas as pl
import jax.experimental.pallas.tpu as pltpu

B, H, SK, D, M = 4, 32, 4096, 128, 512
DC = 512
HKV = 8
NG = B * HKV
KB = 256
NSTEP = SK // KB
NS = 8
CC = 512
SEG = 32 * 1024
PITCH = 36
F32 = jnp.float32
BF16 = jnp.bfloat16
NT = (((1,), (1,)), ((), ()))
NN = (((1,), (0,)), ((), ()))

NLAG = 10
T_CV = 19
T_W = 28
T_A = 36
T_BQ = 11
T_B = 20
T_G = 6
LEAD = 10
LA = 36
NL = 20
OFF = 8
WOFF = 120

(S_AX, S_BX, S_BWQ, S_AWQ, S_AWUK, S_AWUV, S_C, S_K, S_V, S_AO, S_BO) = (0, 1, 2, 3, 4, 5, 6, 10, 12, 14, 21)
NSEM = S_BO + 4
AO_LAST = [(0, 4), (4, 2), (6, 1), (7, 1)]


def _dot(a, b, dims):
    return lax.dot_general(a, b, dims, preferred_element_type=F32)


def _lag(t, extra=0):
    u = t.astype(jnp.uint32)
    for k in range(NLAG):
        u = lax.rem(u, jnp.uint32(900001 - 14 * k))
        if k < extra:
            u = u + jnp.uint32(1)
    if extra:
        u = u - jnp.uint32(extra)
    return u.astype(jnp.int32)


def _lane_tiles(x):
    return [x[:, i:i + 128] for i in range(0, x.shape[1], 128)]


def _kernel(ax_hbm, ckv_hbm, awq_hbm, awuk_hbm, awuv_hbm, awo_hbm, bx_hbm, k_hbm, v_hbm, bwq_hbm, bwo_hbm,
            out_ref,
            ax_buf, bx_buf, bwq_buf, awq_buf, awuk_buf, awuv_buf, c0_buf, c1_buf, c2_buf, c3_buf,
            k0_buf, k1_buf, v0_buf, v1_buf,
            ao0, ao1, ao2, ao3a, ao3b, ao3c, ao3d, bo0, bo1, bo2, bo3,
            q_scr, qa_scr, ctx_scr, ctxh_scr, qb_scr, m_scr, l_scr, acc_scr, ma_scr, la_scr, wf_scr, sems):
    scale = D ** -0.5
    c_bufs = (c0_buf, c1_buf, c2_buf, c3_buf)
    k_bufs = (k0_buf, k1_buf)
    v_bufs = (v0_buf, v1_buf)
    zero = jnp.int32(0)

    class Load:
        def __init__(self, src, dst, sem, nfg=0, s0=0, r0=0, wrap=0, flip=False):
            assert not (nfg and wrap)
            self.src, self.dst, self.sem, self.nfg, self.s0, self.r0 = src, dst, sem, nfg, s0, r0
            self.wrap, self.flip, self.done = wrap, flip, 0
            self.S, self.L, width = dst.shape
            self.seg = SEG // (width * 2)

        def copy(self, s, ns, r, nr):
            return pltpu.make_async_copy(self.src.at[pl.ds(self.s0 + s, ns), pl.ds(self.r0 + r, nr)],
                                         self.dst.at[pl.ds(s, ns), pl.ds(r, nr)], sems.at[self.sem])

        def background(self):
            out = []
            for rnd in range(self.nfg // self.S, self.L // self.seg):
                s = max(self.nfg - rnd * self.S, 0)
                rows = min(self.seg, self.L - self.wrap - rnd * self.seg)
                out.append((self.copy(s, self.S - s, rnd * self.seg, rows), self.S - s))
            if self.wrap:
                out.append((pltpu.make_async_copy(self.src.at[pl.ds(self.s0, self.S), pl.ds(0, self.wrap)],
                                                  self.dst.at[:, pl.ds(self.L - self.wrap, self.wrap)],
                                                  sems.at[self.sem]), 0))
            return out

        def wait(self):
            pltpu.make_async_copy(self.dst, self.dst, sems.at[self.sem]).wait()

        def tick(self, t):
            s = lax.bitwise_and(t, self.S - 1)
            if self.flip:
                s = lax.bitwise_xor(s, self.S - 1)
            rnd = lax.shift_right_logical(t, self.S.bit_length() - 1)
            self.copy(s, 1, pl.multiple_of(rnd * self.seg, self.seg), self.seg).start(priority=0)
            return _lag(t + 1)

    class FlatLoad(Load):
        def __init__(self, src, dst, sem):
            self.src, self.dst, self.sem, self.done = src, dst, sem, 0
            self.wide = dst.shape[1] > D
            self.nfg = 128 if self.wide else 127

        def part(self, *idx):
            return pltpu.make_async_copy(self.src.at[idx], self.dst.at[idx], sems.at[self.sem])

        def background(self):
            if self.wide:
                return []
            tail = WOFF + self.nfg * 128
            return [(self.part(pl.ds(0, WOFF)), 0), (self.part(pl.ds(tail, self.dst.shape[0] - tail)), 0)]

        def tick(self, t):
            s = lax.bitwise_and(t, 7)
            rnd = lax.shift_right_logical(t, 3)
            if self.wide:
                half = self.dst.shape[1] // 2
                i = s * 16 + lax.bitwise_and(rnd + s, 15)
                r = pl.multiple_of(lax.shift_right_logical(i, 1) * 8, 8)
                c = pl.multiple_of(lax.bitwise_and(i, 1) * half, half)
                self.part(pl.ds(r, 8), pl.ds(c, half)).start(priority=0)
            else:
                i = s * 16 + lax.bitwise_xor(rnd, 7 - s)
                self.part(pl.ds(pl.multiple_of(WOFF + i * 128, 8), 128)).start(priority=0)
            return _lag(t + 1, 5)

    class Sched:
        def __init__(self, queue=(), issued=0):
            self.queue, self.issued, self.now = list(queue), issued, 0

        def feed(self, upto):
            while self.queue and self.issued < upto + LA:
                copy, n = self.queue.pop(0)
                copy.start(priority=1)
                self.issued += n

        def count(self, ld, n):
            assert ld.done + n <= ld.nfg
            ld.done += n
            self.now += n

        def ticks(self, ld, t, n):
            for _ in range(n):
                self.feed(self.now)
                self.count(ld, 1)
                t = ld.tick(t)
            return t

        def pump(self, ld, t, n=None):
            n = ld.nfg - ld.done if n is None else n
            self.feed(self.now + n // 2)
            self.count(ld, n)
            return lax.fori_loop(0, n, lambda i, t: ld.tick(t), t) if n else t

    cp_ax = pltpu.make_async_copy(ax_hbm, ax_buf, sems.at[S_AX])
    cp_bx = pltpu.make_async_copy(bx_hbm, bx_buf, sems.at[S_BX])
    awq = FlatLoad(awq_hbm, awq_buf, S_AWQ)
    awuk = FlatLoad(awuk_hbm, awuk_buf, S_AWUK)
    awuv = FlatLoad(awuv_hbm, awuv_buf, S_AWUV)
    bwq = FlatLoad(bwq_hbm, bwq_buf, S_BWQ)
    ckv = [Load(ckv_hbm, c_bufs[k], S_C + k, 128, r0=k * CC) for k in range(4)]
    ao = [Load(awo_hbm, buf, S_AO + g, r0=g * D) for g, buf in enumerate((ao0, ao1, ao2))]
    ao_last = [Load(awo_hbm, buf, S_AO + 3 + i, s0=AO_LAST[i][0], r0=3 * D)
               for i, buf in enumerate((ao3a, ao3b, ao3c, ao3d))]
    bo = [Load(bwo_hbm, buf, S_BO + g, 32 if g < 3 else NL, r0=g * D) for g, buf in enumerate((bo0, bo1, bo2, bo3))]

    def kv_pos(j):
        if isinstance(j, int):
            return dict(r0=SK - KB + OFF, wrap=OFF) if j == 0 else dict(r0=OFF + (j - 1) * KB)
        return dict(r0=pl.multiple_of(OFF + (j - 1) * KB, 8))

    def kc(j, par):
        return Load(k_hbm, k_bufs[par], S_K + par, **kv_pos(j))

    def vc(j, par, nfg=0):
        return Load(v_hbm, v_bufs[par], S_V + par, nfg, flip=True, **kv_pos(j))

    def queue(*loads):
        for ld in loads:
            for copy, _ in ld.background():
                copy.start(priority=1)

    sch = Sched()

    def widen(st, t, w_buf):
        t = sch.ticks(st, t, T_CV)
        for m in range(M):
            wf_scr[pl.ds(m * PITCH, H), :] = w_buf[pl.ds(m * H, H), :].astype(F32)
        return t

    def per_head(st, t, fn):
        t = sch.ticks(st, sch.pump(st, t, 2), T_W)
        for h in range(H):
            fn(h, wf_scr[pl.ds(h, M, stride=PITCH), :].astype(BF16))
        return t

    def q_fn(h, w):
        q_scr[h] = _dot(ax_buf[...], w, NN)

    def qa_fn(h, w):
        qa = _dot(q_scr[h].astype(BF16), w, NT) * scale
        for cc, tile in enumerate(_lane_tiles(qa)):
            qa_scr[cc, pl.ds(h, B, stride=H), :] = tile

    def uv_fn(h, w):
        rows = jnp.concatenate([ctx_scr[cc, pl.ds(h, B, stride=H), :] for cc in range(4)], axis=1)
        ctxh_scr[h] = _dot(rows.astype(BF16), w, NN)

    def a_query(st, t):
        cp_ax.wait()
        return per_head(st, widen(st, t, awq_buf), q_fn)

    def b_query(st, t):
        cp_bx.wait()
        t = sch.ticks(st, t, T_BQ)
        for h, tile in enumerate(_lane_tiles(_dot(bx_buf[...], bwq_buf[...], NN))):
            qb_scr[pl.ds(h, B, stride=H), :] = tile
        return t

    def a_block(st, t, k):
        t = sch.ticks(st, t, T_A)

        def latent(b):
            return c_bufs[k][pl.ds(2 * b, 2)].reshape(2 * CC, DC)

        scores = []
        for b in range(B):
            qa = jnp.concatenate([qa_scr[cc, pl.ds(b * H, H), :] for cc in range(4)], axis=1)
            scores.append(_dot(qa.astype(BF16), latent(b), NT))
        for b in range(B):
            rows = pl.ds(b * H, H)
            m_new = jnp.broadcast_to(jnp.max(scores[b], axis=1, keepdims=True), (H, 128))
            if k > 0:
                m_old = ma_scr[rows, :]
                m_new = jnp.maximum(m_old, m_new)
                alpha = jnp.exp(m_old - m_new)
            e = [jnp.exp(s - m_new) for s in _lane_tiles(scores[b])]
            l = sum(e[1:], e[0])
            ctx = _lane_tiles(_dot(jnp.concatenate(e, axis=1).astype(BF16), latent(b), NN))
            if k > 0:
                l = alpha * la_scr[rows, :] + l
                ctx = [alpha * ctx_scr[cc, rows, :] + ctx[cc] for cc in range(4)]
            if k < 3:
                ma_scr[rows, :] = m_new
                la_scr[rows, :] = l
            else:
                total = jnp.sum(l, axis=1, keepdims=True)
                ctx = [c / total for c in ctx]
            for cc in range(4):
                ctx_scr[cc, rows, :] = ctx[cc]
        return t

    def b_block(st, t, par, nxt, first=False, last=False):
        kc(0, par).wait()
        vc(0, par).wait()
        t = sch.ticks(st, t, T_B + 2 * last)
        low = lax.broadcasted_iota(jnp.int32, (8, 1), 0) < 4

        def paired(x, w_buf, dims):
            out = []
            for p in range(NG // 2):
                x8 = x[8 * p:8 * p + 8, :].astype(BF16)
                out.append(jnp.where(low, _dot(x8, w_buf[2 * p], dims), _dot(x8, w_buf[2 * p + 1], dims)))
            return jnp.concatenate(out, axis=0)

        s = paired(qb_scr[...], k_bufs[par], NT) * scale
        m_new = jnp.broadcast_to(jnp.max(s, axis=1, keepdims=True), (B * H, 128))
        if not first:
            m_old = m_scr[...]
            m_new = jnp.maximum(m_old, m_new)
            alpha = jnp.exp(m_old - m_new)
        e = [jnp.exp(x - m_new) for x in _lane_tiles(s)]
        l = sum(e[1:], e[0])
        acc = paired(jnp.concatenate(e, axis=1), v_bufs[par], NN)
        if not first:
            l = alpha * l_scr[...] + l
            acc = alpha * acc_scr[...] + acc
        if last:
            acc = acc / jnp.sum(l, axis=1, keepdims=True)
        else:
            m_scr[...] = m_new
            l_scr[...] = l
        acc_scr[...] = acc
        queue(*nxt)
        return t

    side = [(bwq, b_query), (awq, a_query), (awuk, lambda st, t: per_head(st, widen(st, t, awuk_buf), qa_fn))]
    side += [(ckv[k], lambda st, t, k=k: a_block(st, t, k)) for k in range(4)] + [(awuv, None)]
    nx = len(side)
    queue(kc(0, 0))
    cp_bx.start(priority=1)
    cp_ax.start(priority=1)
    t = sch.pump(bwq, zero, 16)
    queue(vc(0, 0))
    t = sch.ticks(bwq, t, T_CV + 3)
    wf_scr[...] = jnp.zeros(wf_scr.shape, F32)
    t = sch.pump(bwq, t, 45 - T_CV)
    queue(awq, kc(1, 1), vc(1, 1))
    sch.pump(bwq, t)
    for i in range(1, nx):
        st = side[i][0]
        prev, use_prev = side[i - 1]
        par = (i - 1) % 2
        nxt = [kc(i + 1, par)] + ([side[i + 1][0], vc(i + 1, par)] if i + 1 < nx else [])
        t = sch.pump(st, zero, LEAD)
        prev.wait()
        if i == 1:
            t = b_block(st, use_prev(st, t), par, nxt, first=True)
        else:
            t = use_prev(st, sch.pump(st, b_block(st, t, par, nxt), 2))
        sch.pump(st, t)

    def b_slot(j, par, nxt, extra=None):
        st = vc(j + 1, 1 - par, 2 * NG)
        t = b_block(st, sch.pump(st, zero, LEAD), par, [nxt])
        sch.pump(st, extra(st, t) if extra else t)

    def widen_uv(st, t):
        awuv.wait()
        return widen(st, t, awuv_buf)

    b_slot(nx - 1, 1, kc(nx + 1, 1), widen_uv)
    b_slot(nx, 0, kc(nx + 2, 0), lambda st, t: per_head(st, t, uv_fn))
    b_slot(nx + 1, 1, kc(nx + 3, 1))

    def b_body(i, carry):
        b_slot(2 * i, 0, kc(2 * i + 2, 0))
        b_slot(2 * i + 1, 1, kc(2 * i + 3, 1))
        return carry

    lax.fori_loop(nx // 2 + 1, NSTEP // 2 - 1, b_body, 0)
    b_slot(NSTEP - 2, 0, ao[0])

    sch = Sched(ao[1].background() + ao[2].background() + bo[3].background()
                + [(ld.copy(0, ld.S, 0, ld.L), ld.S * 4) for ld in ao_last], issued=32)
    t = b_block(bo[0], sch.pump(bo[0], zero, LEAD), 1, [], last=True)
    sch.pump(bo[0], t)

    def proj_a(ld, g):
        lhs = jnp.concatenate([ctxh_scr[4 * (ld.s0 + s) + g] for s in range(ld.S)], axis=1)
        return _dot(lhs.astype(BF16), ld.dst[...].reshape(ld.S * D, M), NN)

    def proj_b(ld, g):
        lhs = jnp.concatenate([acc_scr[pl.ds(4 * s + g, B, stride=H), :] for s in range(NS)], axis=1)
        return _dot(lhs.astype(BF16), ld.dst[...].reshape(NS * D, M), NN)

    oa = ob = None
    for g in range(3):
        t = sch.pump(bo[g + 1], zero, LEAD + 2)
        ao[g].wait()
        bo[g].wait()
        t = sch.ticks(bo[g + 1], t, T_G)
        oa = proj_a(ao[g], g) if g == 0 else proj_a(ao[g], g) + oa
        ob = proj_b(bo[g], g) if g == 0 else proj_b(bo[g], g) + ob
        sch.pump(bo[g + 1], t)
    sch.feed(10 ** 9)
    bo[3].wait()
    out_ref[:, M:2 * M] = (proj_b(bo[3], 3) + ob).astype(BF16)
    for ld in ao_last:
        ld.wait()
        oa = proj_a(ld, 3) + oa
    out_ref[:, 0:M] = oa.astype(BF16)


@jax.jit
def pallas_concat_heads__compressed_kv_cla__gqa_block_cached__decode_kernel(
    A_x: jax.Array,
    A_c_kv: jax.Array,
    A_w_q: jax.Array,
    A_w_uk: jax.Array,
    A_w_uv: jax.Array,
    A_w_o: jax.Array,
    B_x: jax.Array,
    B_k_cache: jax.Array,
    B_v_cache: jax.Array,
    B_wq: jax.Array,
    B_wo: jax.Array,
):
    args = (
        A_x.reshape(B, M), A_c_kv.reshape(NS, B * SK // NS, DC),
        A_w_q.reshape(M * H, D), A_w_uk.reshape(DC * H, D), A_w_uv.reshape(DC * H, D),
        A_w_o.reshape(NS, H * D // NS, M),
        B_x.reshape(B, M), B_k_cache.reshape(NG, SK, D), B_v_cache.reshape(NG, SK, D),
        B_wq, B_wo.reshape(NS, H * D // NS, M),
    )
    scratch = (
        [pltpu.VMEM((B, M), BF16)] * 2
        + [pltpu.VMEM((M, H * D), BF16)]
        + [pltpu.VMEM((M * H, D), BF16)] * 3
        + [pltpu.VMEM((NS, CC, DC), BF16)] * 4
        + [pltpu.VMEM((NG, KB, D), BF16)] * 4
        + [pltpu.VMEM((NS, D, M), BF16)] * 3 + [pltpu.VMEM((n, D, M), BF16) for _, n in AO_LAST]
        + [pltpu.VMEM((NS, D, M), BF16)] * 4
        + [pltpu.VMEM((H, B, D), F32),
           pltpu.VMEM((4, B * H, 128), F32), pltpu.VMEM((4, B * H, 128), F32),
           pltpu.VMEM((H, B, D), F32)]
        + [pltpu.VMEM((B * H, D), F32)] * 6
        + [pltpu.VMEM((M * PITCH, D), F32), pltpu.SemaphoreType.DMA((NSEM,))]
    )
    out = pl.pallas_call(
        _kernel,
        in_specs=[pl.BlockSpec(memory_space=pl.ANY)] * 11,
        out_specs=pl.BlockSpec(memory_space=pltpu.VMEM),
        out_shape=jax.ShapeDtypeStruct((B, 2 * M), BF16),
        scratch_shapes=scratch,
        compiler_params=pltpu.CompilerParams(vmem_limit_bytes=80 * 1024 * 1024,
                                             disable_semaphore_checks=True, disable_bounds_checks=True),
    )(*args)
    return out.reshape(B, 1, 2 * M)
```

```python
import jax
import jax.numpy as jnp
from jax import lax
import jax.experimental.pallas as pl
import jax.experimental.pallas.tpu as pltpu

B, H, SK, D, M = 4, 32, 4096, 128, 512
DC = 512
HKV = 8
NG = B * HKV
KB = 256
NSTEP = SK // KB
NS = 8
CC = 512
SEG = 32 * 1024
PITCH = 36
F32 = jnp.float32
BF16 = jnp.bfloat16
NT = (((1,), (1,)), ((), ()))
NN = (((1,), (0,)), ((), ()))

NLAG = 10
T_CV = 32
T_W = 28
T_A = 36
T_BQ = 11
T_B = 20
T_G = 6
LEAD = 10
LA = 36
NL = 20
OFF = 8
WOFF = 120

(S_AX, S_BX, S_BWQ, S_AWQ, S_AWUK, S_AWUV, S_C, S_K, S_V, S_AO, S_BO) = (0, 1, 2, 3, 4, 5, 6, 10, 12, 14, 21)
NSEM = S_BO + 4
AO_LAST = [(0, 4), (4, 2), (6, 1), (7, 1)]


def _dot(a, b, dims):
    return lax.dot_general(a, b, dims, preferred_element_type=F32)


def _lag(t, extra=0):
    u = t.astype(jnp.uint32)
    for k in range(NLAG):
        u = lax.rem(u, jnp.uint32(900001 - 14 * k))
        if k < extra:
            u = u + jnp.uint32(1)
    if extra:
        u = u - jnp.uint32(extra)
    return u.astype(jnp.int32)


def _lane_tiles(x):
    return [x[:, i:i + 128] for i in range(0, x.shape[1], 128)]


def _kernel(ax_hbm, ckv_hbm, awq_hbm, awuk_hbm, awuv_hbm, awo_hbm, bx_hbm, k_hbm, v_hbm, bwq_hbm, bwo_hbm,
            out_ref,
            ax_buf, bx_buf, bwq_buf, awq_buf, awuk_buf, awuv_buf, c0_buf, c1_buf, c2_buf, c3_buf,
            k0_buf, k1_buf, v0_buf, v1_buf,
            ao0, ao1, ao2, ao3a, ao3b, ao3c, ao3d, bo0, bo1, bo2, bo3,
            q_scr, qa_scr, ctx_scr, ctxh_scr, qb_scr, m_scr, l_scr, acc_scr, ma_scr, la_scr, wf_scr, sems):
    scale = D ** -0.5
    c_bufs = (c0_buf, c1_buf, c2_buf, c3_buf)
    k_bufs = (k0_buf, k1_buf)
    v_bufs = (v0_buf, v1_buf)
    zero = jnp.int32(0)

    class Load:
        def __init__(self, src, dst, sem, nfg=0, s0=0, r0=0, wrap=0, flip=False):
            assert not (nfg and wrap)
            self.src, self.dst, self.sem, self.nfg, self.s0, self.r0 = src, dst, sem, nfg, s0, r0
            self.wrap, self.flip, self.done = wrap, flip, 0
            self.S, self.L, width = dst.shape
            self.seg = SEG // (width * 2)

        def copy(self, s, ns, r, nr):
            return pltpu.make_async_copy(self.src.at[pl.ds(self.s0 + s, ns), pl.ds(self.r0 + r, nr)],
                                         self.dst.at[pl.ds(s, ns), pl.ds(r, nr)], sems.at[self.sem])

        def background(self):
            out = []
            for rnd in range(self.nfg // self.S, self.L // self.seg):
                s = max(self.nfg - rnd * self.S, 0)
                rows = min(self.seg, self.L - self.wrap - rnd * self.seg)
                out.append((self.copy(s, self.S - s, rnd * self.seg, rows), self.S - s))
            if self.wrap:
                out.append((pltpu.make_async_copy(self.src.at[pl.ds(self.s0, self.S), pl.ds(0, self.wrap)],
                                                  self.dst.at[:, pl.ds(self.L - self.wrap, self.wrap)],
                                                  sems.at[self.sem]), 0))
            return out

        def wait(self):
            pltpu.make_async_copy(self.dst, self.dst, sems.at[self.sem]).wait()

        def tick(self, t):
            s = lax.bitwise_and(t, self.S - 1)
            if self.flip:
                s = lax.bitwise_xor(s, self.S - 1)
            rnd = lax.shift_right_logical(t, self.S.bit_length() - 1)
            self.copy(s, 1, pl.multiple_of(rnd * self.seg, self.seg), self.seg).start(priority=0)
            return _lag(t + 1)

    class FlatLoad(Load):
        def __init__(self, src, dst, sem):
            self.src, self.dst, self.sem, self.done = src, dst, sem, 0
            self.wide = dst.shape[1] > D
            self.nfg = 128 if self.wide else 127

        def part(self, *idx):
            return pltpu.make_async_copy(self.src.at[idx], self.dst.at[idx], sems.at[self.sem])

        def background(self):
            if self.wide:
                return []
            tail = WOFF + self.nfg * 128
            return [(self.part(pl.ds(0, WOFF)), 0), (self.part(pl.ds(tail, self.dst.shape[0] - tail)), 0)]

        def tick(self, t):
            s = lax.bitwise_and(t, 7)
            rnd = lax.shift_right_logical(t, 3)
            if self.wide:
                half = self.dst.shape[1] // 2
                i = s * 16 + lax.bitwise_and(rnd + s, 15)
                r = pl.multiple_of(lax.shift_right_logical(i, 1) * 8, 8)
                c = pl.multiple_of(lax.bitwise_and(i, 1) * half, half)
                self.part(pl.ds(r, 8), pl.ds(c, half)).start(priority=0)
            else:
                i = s * 16 + lax.bitwise_xor(rnd, 7 - s)
                self.part(pl.ds(pl.multiple_of(WOFF + i * 128, 8), 128)).start(priority=0)
            return _lag(t + 1, 5)

    class Sched:
        def __init__(self, queue=(), issued=0):
            self.queue, self.issued, self.now = list(queue), issued, 0

        def feed(self, upto):
            while self.queue and self.issued < upto + LA:
                copy, n = self.queue.pop(0)
                copy.start(priority=1)
                self.issued += n

        def count(self, ld, n):
            assert ld.done + n <= ld.nfg
            ld.done += n
            self.now += n

        def ticks(self, ld, t, n):
            for _ in range(n):
                self.feed(self.now)
                self.count(ld, 1)
                t = ld.tick(t)
            return t

        def pump(self, ld, t, n=None):
            n = ld.nfg - ld.done if n is None else n
            self.feed(self.now + n // 2)
            self.count(ld, n)
            return lax.fori_loop(0, n, lambda i, t: ld.tick(t), t) if n else t

    cp_ax = pltpu.make_async_copy(ax_hbm, ax_buf, sems.at[S_AX])
    cp_bx = pltpu.make_async_copy(bx_hbm, bx_buf, sems.at[S_BX])
    awq = FlatLoad(awq_hbm, awq_buf, S_AWQ)
    awuk = FlatLoad(awuk_hbm, awuk_buf, S_AWUK)
    awuv = FlatLoad(awuv_hbm, awuv_buf, S_AWUV)
    bwq = FlatLoad(bwq_hbm, bwq_buf, S_BWQ)
    ckv = [Load(ckv_hbm, c_bufs[k], S_C + k, 128, r0=k * CC) for k in range(4)]
    ao = [Load(awo_hbm, buf, S_AO + g, r0=g * D) for g, buf in enumerate((ao0, ao1, ao2))]
    ao_last = [Load(awo_hbm, buf, S_AO + 3 + i, s0=AO_LAST[i][0], r0=3 * D)
               for i, buf in enumerate((ao3a, ao3b, ao3c, ao3d))]
    bo = [Load(bwo_hbm, buf, S_BO + g, 32 if g < 3 else NL, r0=g * D) for g, buf in enumerate((bo0, bo1, bo2, bo3))]

    def kv_pos(j):
        if isinstance(j, int):
            return dict(r0=SK - KB + OFF, wrap=OFF) if j == 0 else dict(r0=OFF + (j - 1) * KB)
        return dict(r0=pl.multiple_of(OFF + (j - 1) * KB, 8))

    def kc(j, par):
        return Load(k_hbm, k_bufs[par], S_K + par, **kv_pos(j))

    def vc(j, par, nfg=0):
        return Load(v_hbm, v_bufs[par], S_V + par, nfg, flip=True, **kv_pos(j))

    def queue(*loads):
        for ld in loads:
            for copy, _ in ld.background():
                copy.start(priority=1)

    sch = Sched()

    def widen(st, t, w_buf):
        n = M // T_CV

        def body(i, t):
            src = w_buf[pl.ds(pl.multiple_of(i * (n * H), n * H), n * H), :].astype(F32)
            dst = wf_scr.at[pl.ds(pl.multiple_of(i * (n * PITCH), 8), n * PITCH)]
            for m in range(n):
                dst[pl.ds(m * PITCH, H), :] = src[m * H:(m + 1) * H]
            return st.tick(t)

        sch.count(st, T_CV)
        return lax.fori_loop(0, T_CV, body, t)

    def per_head(st, t, fn):
        t = sch.ticks(st, t, T_W)
        for h in range(H):
            fn(h, wf_scr[pl.ds(h, M, stride=PITCH), :].astype(BF16))
        return t

    def q_fn(h, w):
        q_scr[h] = _dot(ax_buf[...], w, NN)

    def qa_fn(h, w):
        qa = _dot(q_scr[h].astype(BF16), w, NT) * scale
        for cc, tile in enumerate(_lane_tiles(qa)):
            qa_scr[cc, pl.ds(h, B, stride=H), :] = tile

    def uv_fn(h, w):
        rows = jnp.concatenate([ctx_scr[cc, pl.ds(h, B, stride=H), :] for cc in range(4)], axis=1)
        ctxh_scr[h] = _dot(rows.astype(BF16), w, NN)

    def a_query(st, t):
        cp_ax.wait()
        return per_head(st, widen(st, t, awq_buf), q_fn)

    def b_query(st, t):
        cp_bx.wait()
        t = sch.ticks(st, t, T_BQ)
        for h, tile in enumerate(_lane_tiles(_dot(bx_buf[...], bwq_buf[...], NN))):
            qb_scr[pl.ds(h, B, stride=H), :] = tile
        return t

    def a_block(st, t, k):
        t = sch.ticks(st, t, T_A)

        def latent(b):
            return c_bufs[k][pl.ds(2 * b, 2)].reshape(2 * CC, DC)

        scores = []
        for b in range(B):
            qa = jnp.concatenate([qa_scr[cc, pl.ds(b * H, H), :] for cc in range(4)], axis=1)
            scores.append(_dot(qa.astype(BF16), latent(b), NT))
        for b in range(B):
            rows = pl.ds(b * H, H)
            m_new = jnp.broadcast_to(jnp.max(scores[b], axis=1, keepdims=True), (H, 128))
            if k > 0:
                m_old = ma_scr[rows, :]
                m_new = jnp.maximum(m_old, m_new)
                alpha = jnp.exp(m_old - m_new)
            e = [jnp.exp(s - m_new) for s in _lane_tiles(scores[b])]
            l = sum(e[1:], e[0])
            ctx = _lane_tiles(_dot(jnp.concatenate(e, axis=1).astype(BF16), latent(b), NN))
            if k > 0:
                l = alpha * la_scr[rows, :] + l
                ctx = [alpha * ctx_scr[cc, rows, :] + ctx[cc] for cc in range(4)]
            if k < 3:
                ma_scr[rows, :] = m_new
                la_scr[rows, :] = l
            else:
                total = jnp.sum(l, axis=1, keepdims=True)
                ctx = [c / total for c in ctx]
            for cc in range(4):
                ctx_scr[cc, rows, :] = ctx[cc]
        return t

    def b_block(st, t, par, nxt, first=False, last=False):
        kc(0, par).wait()
        vc(0, par).wait()
        t = sch.ticks(st, t, T_B + 2 * last)
        low = lax.broadcasted_iota(jnp.int32, (8, 1), 0) < 4

        def paired(x, w_buf, dims):
            out = []
            for p in range(NG // 2):
                x8 = x[8 * p:8 * p + 8, :].astype(BF16)
                out.append(jnp.where(low, _dot(x8, w_buf[2 * p], dims), _dot(x8, w_buf[2 * p + 1], dims)))
            return jnp.concatenate(out, axis=0)

        s = paired(qb_scr[...], k_bufs[par], NT) * scale
        m_new = jnp.broadcast_to(jnp.max(s, axis=1, keepdims=True), (B * H, 128))
        if not first:
            m_old = m_scr[...]
            m_new = jnp.maximum(m_old, m_new)
            alpha = jnp.exp(m_old - m_new)
        e = [jnp.exp(x - m_new) for x in _lane_tiles(s)]
        l = sum(e[1:], e[0])
        acc = paired(jnp.concatenate(e, axis=1), v_bufs[par], NN)
        if not first:
            l = alpha * l_scr[...] + l
            acc = alpha * acc_scr[...] + acc
        if last:
            acc = acc / jnp.sum(l, axis=1, keepdims=True)
        else:
            m_scr[...] = m_new
            l_scr[...] = l
        acc_scr[...] = acc
        queue(*nxt)
        return t

    side = [(bwq, b_query), (awq, a_query), (awuk, lambda st, t: per_head(st, widen(st, t, awuk_buf), qa_fn))]
    side += [(ckv[k], lambda st, t, k=k: a_block(st, t, k)) for k in range(4)] + [(awuv, None)]
    nx = len(side)
    queue(kc(0, 0))
    cp_bx.start(priority=1)
    cp_ax.start(priority=1)
    t = sch.pump(bwq, zero, 16)
    queue(vc(0, 0))
    t = sch.ticks(bwq, t, 22)
    wf_scr[...] = jnp.zeros(wf_scr.shape, F32)
    t = sch.pump(bwq, t, 26)
    queue(awq, kc(1, 1), vc(1, 1))
    sch.pump(bwq, t)
    for i in range(1, nx):
        st = side[i][0]
        prev, use_prev = side[i - 1]
        par = (i - 1) % 2
        nxt = [kc(i + 1, par)] + ([side[i + 1][0], vc(i + 1, par)] if i + 1 < nx else [])
        t = sch.pump(st, zero, LEAD)
        prev.wait()
        if i == 1:
            t = b_block(st, use_prev(st, t), par, nxt, first=True)
        else:
            t = use_prev(st, sch.pump(st, b_block(st, t, par, nxt), 2))
        sch.pump(st, t)

    def b_slot(j, par, nxt, extra=None):
        st = vc(j + 1, 1 - par, 2 * NG)
        t = b_block(st, sch.pump(st, zero, LEAD), par, [nxt])
        sch.pump(st, extra(st, t) if extra else t)

    def widen_uv(st, t):
        awuv.wait()
        return widen(st, t, awuv_buf)

    b_slot(nx - 1, 1, kc(nx + 1, 1), widen_uv)
    b_slot(nx, 0, kc(nx + 2, 0), lambda st, t: per_head(st, sch.pump(st, t, 2), uv_fn))
    b_slot(nx + 1, 1, kc(nx + 3, 1))

    def b_body(i, carry):
        b_slot(2 * i, 0, kc(2 * i + 2, 0))
        b_slot(2 * i + 1, 1, kc(2 * i + 3, 1))
        return carry

    lax.fori_loop(nx // 2 + 1, NSTEP // 2 - 1, b_body, 0)
    b_slot(NSTEP - 2, 0, ao[0])

    sch = Sched(ao[1].background() + ao[2].background() + bo[3].background()
                + [(ld.copy(0, ld.S, 0, ld.L), ld.S * 4) for ld in ao_last], issued=32)
    t = b_block(bo[0], sch.pump(bo[0], zero, LEAD), 1, [], last=True)
    sch.pump(bo[0], t)

    def proj_a(ld, g):
        lhs = jnp.concatenate([ctxh_scr[4 * (ld.s0 + s) + g] for s in range(ld.S)], axis=1)
        return _dot(lhs.astype(BF16), ld.dst[...].reshape(ld.S * D, M), NN)

    def proj_b(ld, g):
        lhs = jnp.concatenate([acc_scr[pl.ds(4 * s + g, B, stride=H), :] for s in range(NS)], axis=1)
        return _dot(lhs.astype(BF16), ld.dst[...].reshape(NS * D, M), NN)

    oa = ob = None
    for g in range(3):
        t = sch.pump(bo[g + 1], zero, LEAD + 2)
        ao[g].wait()
        bo[g].wait()
        t = sch.ticks(bo[g + 1], t, T_G)
        oa = proj_a(ao[g], g) if g == 0 else proj_a(ao[g], g) + oa
        ob = proj_b(bo[g], g) if g == 0 else proj_b(bo[g], g) + ob
        sch.pump(bo[g + 1], t)
    sch.feed(10 ** 9)
    bo[3].wait()
    out_ref[:, M:2 * M] = (proj_b(bo[3], 3) + ob).astype(BF16)
    for ld in ao_last:
        ld.wait()
        oa = proj_a(ld, 3) + oa
    out_ref[:, 0:M] = oa.astype(BF16)


@jax.jit
def pallas_concat_heads__compressed_kv_cla__gqa_block_cached__decode_kernel(
    A_x: jax.Array,
    A_c_kv: jax.Array,
    A_w_q: jax.Array,
    A_w_uk: jax.Array,
    A_w_uv: jax.Array,
    A_w_o: jax.Array,
    B_x: jax.Array,
    B_k_cache: jax.Array,
    B_v_cache: jax.Array,
    B_wq: jax.Array,
    B_wo: jax.Array,
):
    args = (
        A_x.reshape(B, M), A_c_kv.reshape(NS, B * SK // NS, DC),
        A_w_q.reshape(M * H, D), A_w_uk.reshape(DC * H, D), A_w_uv.reshape(DC * H, D),
        A_w_o.reshape(NS, H * D // NS, M),
        B_x.reshape(B, M), B_k_cache.reshape(NG, SK, D), B_v_cache.reshape(NG, SK, D),
        B_wq, B_wo.reshape(NS, H * D // NS, M),
    )
    scratch = (
        [pltpu.VMEM((B, M), BF16)] * 2
        + [pltpu.VMEM((M, H * D), BF16)]
        + [pltpu.VMEM((M * H, D), BF16)] * 3
        + [pltpu.VMEM((NS, CC, DC), BF16)] * 4
        + [pltpu.VMEM((NG, KB, D), BF16)] * 4
        + [pltpu.VMEM((NS, D, M), BF16)] * 3 + [pltpu.VMEM((n, D, M), BF16) for _, n in AO_LAST]
        + [pltpu.VMEM((NS, D, M), BF16)] * 4
        + [pltpu.VMEM((H, B, D), F32),
           pltpu.VMEM((4, B * H, 128), F32), pltpu.VMEM((4, B * H, 128), F32),
           pltpu.VMEM((H, B, D), F32)]
        + [pltpu.VMEM((B * H, D), F32)] * 6
        + [pltpu.VMEM((M * PITCH, D), F32), pltpu.SemaphoreType.DMA((NSEM,))]
    )
    out = pl.pallas_call(
        _kernel,
        in_specs=[pl.BlockSpec(memory_space=pl.ANY)] * 11,
        out_specs=pl.BlockSpec(memory_space=pltpu.VMEM),
        out_shape=jax.ShapeDtypeStruct((B, 2 * M), BF16),
        scratch_shapes=scratch,
        compiler_params=pltpu.CompilerParams(vmem_limit_bytes=80 * 1024 * 1024,
                                             disable_semaphore_checks=True, disable_bounds_checks=True),
    )(*args)
    return out.reshape(B, 1, 2 * M)
```
